```python
import os as _os
_os.environ.setdefault("JAX_PLATFORMS", "cpu")
import jax
import jax.numpy as jnp

def _softmax(x, axis=-1):
    return jax.nn.softmax(x, axis=axis)
def _gelu(x):
    return jax.nn.gelu(x, approximate=True)
def _silu(x):
    return jax.nn.silu(x)
def _sigmoid(x):
    return jax.nn.sigmoid(x)
def _layernorm(x, axis=-1, eps=1e-5):
    m = jnp.mean(x, axis=axis, keepdims=True)
    v = jnp.var(x, axis=axis, keepdims=True)
    return (x - m) / jnp.sqrt(v + eps)
def _scatter_add(tgt, idx, src, axis=0):
    return tgt.at[idx].add(src)
def _segment_sum(src, seg, n):
    return jax.ops.segment_sum(src, seg, n)
class _Rng:
    def __init__(self, key):
        self._k = key
    def _next(self):
        self._k, sub = jax.random.split(self._k)
        return sub
    def normal(self, shape):
        return jax.random.normal(self._next(), shape, dtype=jnp.bfloat16)
    def randint(self, lo, hi, shape):
        return jax.random.randint(self._next(), shape, lo, hi, dtype=jnp.int32)
    def uniform(self, shape, lo=0.0, hi=1.0):
        return jax.random.uniform(self._next(), shape, jnp.bfloat16, lo, hi)
    def permutation(self, n):
        return jax.random.permutation(self._next(), n)


kernel_name = 'interleave_layers__spectral_gfnet__linear_attn_block__prompt'

def setup_inputs():
    _rng = _Rng(jax.random.key(int.from_bytes(__import__("os").urandom(4), "little")))
    _w = (lambda a: (lambda t: t.astype(jnp.bfloat16) if jnp.issubdtype(t.dtype, jnp.floating) else t)(jnp.asarray(a)))
    def _A_setup():
        B, S, D = 1, 2048, 640
        Df = D // 2 + 1
        return {
            "x": _w((lambda *s: _rng.normal(s) * 0.05)(B, S, D)),
            "w_r": _w((lambda *s: _rng.normal(s) * 0.4)(S, Df) * 0.02),
            "w_i": _w((lambda *s: _rng.normal(s) * 0.4)(S, Df) * 0.02),
        }
    _A_in = _A_setup()

    def _B_setup():
        B, S, D = 1, 2048, 640
        return {
            "x": _w((lambda *s: _rng.normal(s) * 0.05)(B, S, D)),
            "wqkv": _w((lambda *s: _rng.normal(s) * 0.05)(D, 3 * D)),
            "wo": _w((lambda *s: _rng.normal(s) * 0.05)(D, D)),
        }
    _B_in = _B_setup()

    return {
        "A_x": _A_in["x"],
        "A_w_r": _A_in["w_r"],
        "A_w_i": _A_in["w_i"],
        "B_x": _B_in["x"],
        "B_wqkv": _B_in["wqkv"],
        "B_wo": _B_in["wo"],
    }

def reference(A_x, A_w_r, A_w_i, B_x, B_wqkv, B_wo):
    def _A_ref(x, w_r, w_i):
        B, S, D = x.shape
        X = (lambda x, axes=(-2,-1): jnp.fft.rfft2(x.astype(jnp.float32), axes=axes))(x, axes=(-2, -1))
        W = w_r + 1j * w_i
        X = X * W
        y = (lambda x, s, axes=(-2,-1): jnp.fft.irfft2(x, s=s, axes=axes).astype(jnp.bfloat16))(X, (S, D), axes=(-2, -1))
        return y

    def _B_ref(x, wqkv, wo):
        B, S, D = x.shape
        H = 32; Dh = D // H
        qkv = (lambda x, *d: x.transpose(*d))((x @ wqkv).reshape(B, S, 3, H, Dh), 2, 0, 3, 1, 4)
        q, k, v = qkv[0], qkv[1], qkv[2]
        phi = lambda t: jnp.where(t > 0, t + 1, jnp.exp(t)) + 1e-6
        pq, pk = phi(q), phi(k)
        kv = jnp.einsum("bhsd,bhse->bhde", pk, v)
        z = jnp.einsum("bhsd->bhd", pk)
        num = jnp.einsum("bhqd,bhde->bhqe", pq, kv)
        den = jnp.einsum("bhqd,bhd->bhq", pq, z)[..., None] + 1e-6
        o = num / den
        return (lambda x, *d: x.transpose(*d))(o, 0, 2, 1, 3).reshape(B, S, D) @ wo

    x = A_x
    x = x + _A_ref(_layernorm(x, axis=-1), A_w_r, A_w_i)
    x = x + _B_ref(_layernorm(x, axis=-1), B_wqkv, B_wo)
    x = x + _A_ref(_layernorm(x, axis=-1), A_w_r, A_w_i)
    x = x + _B_ref(_layernorm(x, axis=-1), B_wqkv, B_wo)
    return x
```

```python
import numpy as np
import jax
import jax.numpy as jnp
from jax import lax
import jax.experimental.pallas as pl
import jax.experimental.pallas.tpu as pltpu

S, D, H, DH = 2048, 640, 32, 20
DF = D // 2 + 1
R1, R2 = 32, 64
G = 8
NC = 4
NS = R2 // (G * NC)
CH = R1 * G * NS
NT = D // 128

_C5 = float(np.sqrt(5.0) / 4.0)
_R5 = float(np.sin(4 * np.pi / 5) / np.sin(2 * np.pi / 5))
_CLASSES = ((0, 5), (4, 6), (1, 9), (2, 8), (3, 7))


def _cmul(re, im, ang):
    c, s = float(np.cos(ang)), float(np.sin(ang))
    if abs(abs(c) - abs(s)) < 1e-12:
        if c * s > 0:
            return (re - im) * c, (re + im) * c
        return (re + im) * c, (im - re) * c
    return re * c - im * s, re * s + im * c


def _cplx_fwd(u, th):
    n = len(u)
    if n == 1:
        return [(th, u[0])]
    h = n // 2
    v = [_cmul(re, im, th / 2) for re, im in u[h:]]
    a = [(p[0] + q[0], p[1] + q[1]) for p, q in zip(u[:h], v)]
    b = [(p[0] - q[0], p[1] - q[1]) for p, q in zip(u[:h], v)]
    return _cplx_fwd(a, th / 2) + _cplx_fwd(b, th / 2 + np.pi)


def _cplx_bwd(g, th):
    n = len(g)
    if n == 1:
        return list(g)
    h = n // 2
    a, b = _cplx_bwd(g[:h], th / 2), _cplx_bwd(g[h:], th / 2 + np.pi)
    lo = [(p[0] + q[0], p[1] + q[1]) for p, q in zip(a, b)]
    hi = [_cmul(p[0] - q[0], p[1] - q[1], -th / 2) for p, q in zip(a, b)]
    return lo + hi


def _real_fwd(x):
    n = len(x)
    if n == 2:
        return [(0.0, (x[0], x[1]))]
    h, q = n // 2, n // 4
    a = [x[j] + x[j + h] for j in range(h)]
    b = [x[j] - x[j + h] for j in range(h)]
    return _real_fwd(a) + _cplx_fwd([(b[j], b[j + q]) for j in range(q)], np.pi / 2)


def _real_bwd(g):
    if len(g) == 1:
        return list(g[0])
    h = len(g) // 2
    a = _real_bwd(g[:h])
    u = _cplx_bwd(g[h:], np.pi / 2)
    b = [p[0] for p in u] + [p[1] for p in u]
    return [p + q for p, q in zip(a, b)] + [p - q for p, q in zip(a, b)]


def _r10_fwd(x, sel, roll):
    x = [sel(x[j], x[(j + 2) % 5]) for j in range(5)]
    t1, t2, t3, t4 = x[1] + x[4], x[2] + x[3], x[1] - x[4], x[2] - x[3]
    t5 = t1 + t2
    m1, m2 = x[0] - t5 * 0.25, (t1 - t2) * _C5
    out = [x[0] + t5]
    for re, im in ((m1 + m2, t3 + t4 * _R5), (m1 - m2, t3 * _R5 - t4)):
        a, b = sel(re, im), roll(sel(im, re))
        out += [a + b, a - b]
    return out


def _r10_bwd(g, sel, roll):
    re, im = [], []
    for u, v in ((g[1], g[2]), (g[3], g[4])):
        a, b = u + v, roll(u - v)
        re.append(sel(a, b))
        im.append(sel(b, a))
    m1, e = re[0] + re[1], (re[0] - re[1]) * _C5
    t5 = g[0] - m1 * 0.25
    t1, t2 = t5 + e, t5 - e
    t3, t4 = im[0] + im[1] * _R5, im[0] * _R5 - im[1]
    x = [g[0] + m1, t1 + t3, t2 + t4, t2 - t4, t1 - t3]
    return [sel(x[j], x[(j + 3) % 5]) for j in range(5)]


def _build_constants():
    lane = np.arange(128)
    grp = [np.concatenate([c + 10 * np.arange(32) for c in cls]) for cls in _CLASSES]
    d = np.arange(D)[:, None]
    cols = []
    for g, kd in enumerate(grp):
        c, s = np.cos(2 * np.pi * d * kd / D), np.sin(2 * np.pi * d * kd / D)
        if g == 0:
            s[:, 0] = np.cos(np.pi * d[:, 0])
        cols.append(np.concatenate([s, c] if g in (2, 4) else [c, s], axis=1))
    eye = np.eye(D)
    net = np.concatenate(_r10_fwd(
        [eye[:, 128 * j:128 * j + 128] for j in range(NT)],
        lambda a, b: np.where(lane < 64, a, b), lambda a: np.roll(a, 64, axis=1)), axis=1)
    bd = np.linalg.solve(net, np.concatenate(cols, axis=1))
    fd = np.stack([bd[128 * j:128 * j + 128, 128 * j:128 * j + 128] for j in range(NT)])
    assert abs(np.abs(bd).sum() - np.abs(fd).sum()) < 1e-6
    dmat = np.concatenate([fd, fd.transpose(0, 2, 1) / D])

    leaves = [int(round(th * R1 / (2 * np.pi))) for th, _ in _real_fwd(list(np.eye(R1)))]
    k1 = [min(m, R1 - m) for m in leaves]
    pos = np.arange(128)
    part, n2 = (pos // G) % 2, (pos // (2 * G)) * G + pos % G
    fs = []
    for m, kk in zip(leaves, k1):
        ks = (16 * np.arange(R2) if m == 0 else kk + R1 * np.arange(R2))[:, None]
        if m == 0:
            ph = 2 * np.pi * ks * (n2 + R2 * part) / S
            c, s = np.cos(ph), np.sin(ph)
            s[0] = np.cos(np.pi * n2)
        else:
            sg = 1.0 if m == kk else -1.0
            ph = 2 * np.pi * ks * n2 / S
            c = np.where(part == 0, np.cos(ph), -sg * np.sin(ph))
            s = np.where(part == 0, np.sin(ph), sg * np.cos(ph))
        fs.append(np.concatenate([c, s]))
    fs = np.stack(fs)
    smat = np.concatenate([fs, fs.transpose(0, 2, 1) * (2.0 / S)])

    have = np.concatenate([R1 * np.arange(R2), 16 + R1 * (R2 - 1 - np.arange(R2))])
    want = np.concatenate([16 * np.arange(R2), S // 2 + 16 * ((R2 - np.arange(R2)) % R2)])
    p0 = (want[:, None] == have[None, :]).astype(np.float64)

    mats = np.concatenate([dmat, smat, p0[None]]).astype(jnp.bfloat16)
    return mats, k1


_MATS, _K1 = _build_constants()
_DF, _DI, _SF, _SI, _P0 = 0, NT, 2 * NT, 2 * NT + 16, 2 * NT + 32

F32, BF16, I32 = jnp.float32, jnp.bfloat16, jnp.int32
PITCH = 72
RB = 16
_WIN = ((0, 144), (112, 272), (240, 400), (368, 528), (496, 640))


def _dot(a, b):
    return jnp.dot(a, b, preferred_element_type=F32)


def _dot_nt(a, b):
    return lax.dot_general(a, b, (((1,), (1,)), ((), ())), preferred_element_type=F32)


def _sel(a, b):
    return jnp.where(lax.broadcasted_iota(I32, a.shape, 1) < 64, a, b)


def _roll(a):
    return pltpu.roll(a, 64, 1)


def _tiles(a):
    return [a[:, 128 * j:128 * j + 128] for j in range(a.shape[1] // 128)]


def _cat(a, axis=0):
    return a[0] if len(a) == 1 else jnp.concatenate(a, axis=axis)


def _words(a):
    return pltpu.bitcast(a, I32)


def _phi(t):
    return jnp.where(t > 0, t + 1.0, jnp.exp(t)) + 1e-6


def _ln(x):
    mean = jnp.sum(x[0] + x[1] + x[2] + x[3] + x[4], axis=1, keepdims=True) * (1.0 / D)
    x = [a - mean for a in x]
    sq = x[0] * x[0] + x[1] * x[1] + x[2] * x[2] + x[3] * x[3] + x[4] * x[4]
    r = lax.rsqrt(jnp.sum(sq, axis=1, keepdims=True) * (1.0 / D) + 1e-5)
    return [a * r for a in x]


def _kernel(x_hbm, wr_hbm, wi_hbm, wqkv_hbm, wo_hbm, mats_hbm, o_hbm,
            xio, xres, xn, z, zi, wraw, wtmp, wbuf, wqkv, wo, wqp, wkt,
            gacc, zacc, macc, mp, zrow, mats, sems):
    rows = G * NS

    def x_copy(c):
        return pltpu.make_async_copy(
            x_hbm.at[:, pl.ds(pl.multiple_of(c * rows, rows), rows), :], xio.at[c], sems.at[c])

    def o_copy(c):
        return pltpu.make_async_copy(
            xio.at[c], o_hbm.at[:, pl.ds(pl.multiple_of(c * rows, rows), rows), :], sems.at[c])

    other = [pltpu.make_async_copy(s, d, sems.at[NC + i]) for i, (s, d) in enumerate((
        (mats_hbm, mats), (wr_hbm, wraw.at[0]), (wi_hbm, wraw.at[1]),
        (wqkv_hbm, wqkv), (wo_hbm, wo)))]
    x_copy(0).start()
    other[0].start()
    for c in range(1, NC):
        x_copy(c).start()
    for cp in other[1:]:
        cp.start()

    def spec_fwd(c, blocks):
        t = [_r10_fwd(_ln(_tiles(b)), _sel, _roll) for b in blocks]
        y = [_dot(_cat([b[j].astype(BF16) for b in t]), mats[_DF + j]) for j in range(NT)]
        for u in range(NS):
            w = []
            for j in range(NT):
                v = _real_fwd([y[j][(u * R1 + n) * G:(u * R1 + n + 1) * G] for n in range(R1)])
                w.append([_cat(list(p)).astype(BF16) for _, p in v])
            r0 = pl.multiple_of((c * NS + u) * 2 * G, 2 * G)
            for s in range(16):
                out = [w[0][s]]
                for j in (1, 3):
                    a, b = _words(w[j][s]), _words(w[j + 1][s])
                    out += [pltpu.bitcast(_sel(a, b), BF16),
                            pltpu.bitcast(_roll(_sel(b, a)), BF16)]
                z[s, pl.ds(r0, 2 * G), :] = _cat(out, 1)

    def spec_bwd(c):
        t = [[] for _ in range(NT)]
        for u in range(NS):
            r0 = pl.multiple_of((c * NS + u) * 2 * G, 2 * G)
            w = []
            for j in range(NT):
                ls = slice(128 * j, 128 * j + 128)
                v = _real_bwd([(zi[s, pl.ds(r0, G), ls], zi[s, pl.ds(r0 + G, G), ls])
                               for s in range(16)])
                w.append([_cat(v[2 * n:2 * n + 2]).astype(BF16) for n in range(16)])
            for n in range(16):
                t[0].append(w[0][n])
                for j in (1, 3):
                    a, b = _words(w[j][n]), _roll(_words(w[j + 1][n]))
                    t[j].append(pltpu.bitcast(_sel(a, b), BF16))
                    t[j + 1].append(pltpu.bitcast(_sel(b, a), BF16))
        y = [_dot(_cat(t[j]), mats[_DI + j]) for j in range(NT)]
        for r in range(0, CH, RB):
            d = _r10_bwd([a[r:r + RB] for a in y], _sel, _roll)
            x = [a + b for a, b in zip(_tiles(xres[c, r:r + RB, :]), d)]
            xres[c, r:r + RB, :] = _cat(x, 1)
            xn[c, r:r + RB, :] = _cat(_ln(x), 1).astype(BF16)

    def prep_filter():
        hi = jnp.int32(-65536)
        for t in range(S // 128):
            ls = slice(128 * t, 128 * t + 128)
            a, b = _words(wraw[0, 0:D // 2, ls]), _words(wraw[1, 0:D // 2, ls])
            wtmp[t, 0] = (a << 16) | (b & 0xFFFF)
            wtmp[t, 1] = (a & hi) | lax.shift_right_logical(b, 16)
        for t in range(S // 128):
            ls = slice(128 * t, 128 * t + 128)
            last = _words(wraw[0, D // 2:DF, ls].astype(F32)) | lax.shift_right_logical(
                _words(wraw[1, D // 2:DF, ls].astype(F32)), 16)
            cls = lambda c: wtmp[t, c % 2, pl.ds(c // 2, 32, stride=5), :]
            c0, c5 = cls(0), cls(5)
            c0n = jnp.where(lax.broadcasted_iota(I32, c0.shape, 0) == 0, last, c0)
            src = [[c0, c5, c0n, c5]] + [
                [cls(c) for c in _CLASSES[j] + _CLASSES[j + 1]] for j in (1, 3)]
            for j in range(3):
                w = _cat(src[j]).T
                for i in range(16):
                    k2, k1 = 4 * t + i // 4, 8 * (i % 4)
                    pos = k2 if k1 < 16 else R2 - 1 - k2
                    wbuf[j, pl.ds(k1 * PITCH + pos, 8, stride=PITCH), :] = w[8 * i:8 * i + 8]
        for j in range(3):
            w = _cat([wbuf[j, 0:R2, :], wbuf[j, 16 * PITCH:16 * PITCH + R2, :]])
            re = _dot(mats[_P0], pltpu.bitcast(w & hi, F32).astype(BF16))
            im = _dot(mats[_P0], pltpu.bitcast(w << 16, F32).astype(BF16))
            w = _words(re) | lax.shift_right_logical(_words(im), 16)
            wbuf[j, 0:R2, :] = w[:R2]
            wbuf[j, 16 * PITCH:16 * PITCH + R2, :] = w[R2:]

    def prep_weights():
        r = lax.broadcasted_iota(I32, (D, D), 0)
        c = lax.broadcasted_iota(I32, (D, D), 1)
        perm = jnp.where(r == (c & (H - 1)) * DH + (c >> 5), 1.0, 0.0).astype(BF16)
        wqp[...] = _dot(wqkv[:, 0:D], perm).astype(BF16)
        wkt[...] = wqkv[:, D:2 * D].astype(F32).T.astype(BF16)

    def spec_mid():
        lane = lax.broadcasted_iota(I32, (R2, 128), 1)
        edge = (lane & 63) == 0
        sgn = jnp.where(lane < 64, -1.0, 1.0)
        s0 = jnp.where(edge, 0.0, sgn)
        for s in range(16):
            k1 = _K1[s]
            p1, p2 = k1 * PITCH, (R1 - k1 if k1 else 16) * PITCH
            if k1:
                m = lambda a: a
            else:
                row0 = lax.broadcasted_iota(I32, (R2, 128), 0) == 0
                m = lambda a: jnp.where(row0, 0.0, a)

            def coef(j, p):
                w = wbuf[j, p:p + R2, :]
                return pltpu.bitcast(w & jnp.int32(-65536), F32), pltpu.bitcast(w << 16, F32)

            x = _dot(mats[_SF + s], z[s])
            tc, ts = _tiles(x[:R2]), _tiles(x[R2:])
            a, b = _sel(tc[0], ts[0]), _sel(ts[0], tc[0])
            re, im = a + m(_roll(a) * s0), m(b) - _roll(b) * s0
            (a1, b1), (a2, b2) = coef(0, p1), coef(0, p2)
            cr = jnp.where(edge, (a1 + a2) * 0.5, _sel(a1, a2))
            ci = jnp.where(edge, (b2 - b1) * (sgn * 0.5), _sel(b1, b2))
            re, im = cr * re + ci * im, cr * im - ci * re
            an, bn = re - m(_roll(re) * s0), m(im) + _roll(im) * s0
            if not k1:
                an = jnp.where(row0 & edge, a * _sel(a1, a2) * 0.5, an)
                bn = jnp.where(row0 & edge, b * _sel(a2, a1) * 0.5, bn)
            oc, os_ = [_sel(an, bn)], [_sel(bn, an)]
            for j in (1, 3):
                cc, cs, sc, ss = tc[j], tc[j + 1], ts[j], ts[j + 1]
                r1, n1, r2, n2 = cc - m(ss), cs + m(sc), m(cc) + ss, m(cs) - sc
                (a1, b1), (a2, b2) = coef((j + 1) // 2, p1), coef((j + 1) // 2, p2)
                r1, n1 = a1 * r1 + b1 * n1, a1 * n1 - b1 * r1
                r2, n2 = a2 * r2 + b2 * n2, a2 * n2 - b2 * r2
                oc += [r1 + m(r2), n1 + m(n2)]
                os_ += [m(n1) - n2, r2 - m(r1)]
            y = _cat([_cat(oc, 1), _cat(os_, 1)]).astype(BF16)
            zi[s] = _dot(mats[_SI + s], y)

    def attn_stats(c):
        a = xn[c]
        pk = _phi(_dot_nt(wkt[...], a))
        t = _tiles(pk)
        zacc[...] += sum(t[1:], t[0])
        gacc[...] += _dot(pk.astype(BF16), a)

    def attn_mix():
        macc[...] = jnp.zeros(macc.shape, F32)
        for j, (r0, r1) in enumerate(_WIN):
            kv = _dot(gacc[r0:r1, :].astype(BF16), wqkv[:, 2 * D + 128 * j:2 * D + 128 * j + 128])
            hr = ((lax.broadcasted_iota(I32, kv.shape, 0) + r0) * 3277) >> 16
            hc = ((lax.broadcasted_iota(I32, kv.shape, 1) + 128 * j) * 3277) >> 16
            m = _dot(jnp.where(hr == hc, kv, 0.0).astype(BF16), wo[128 * j:128 * j + 128, :])
            for t, a in enumerate(_tiles(m)):
                macc[t, r0:r1, :] += a
        for t in range(NT):
            mp[:, 128 * t:128 * t + 128] = _cat(
                [macc[t, pl.ds(d, H, stride=DH), :] for d in range(DH)]).astype(BF16)
        zp = _cat([zacc[pl.ds(d, H, stride=DH), :] for d in range(DH)])
        zrow[...] = jnp.broadcast_to(jnp.sum(zp.T, axis=0, keepdims=True), zrow.shape)

    def attn_out(c):
        q = _dot(xn[c], wqp[...])
        zt = _tiles(_cat([zrow[...]] * (RB // 8)))
        pn = []
        for r in range(0, CH, RB):
            p = _tiles(_phi(q[r:r + RB]))
            den = p[0] * zt[0] + p[1] * zt[1] + p[2] * zt[2] + p[3] * zt[3] + p[4] * zt[4]
            den = den + _roll(den)
            den = den + pltpu.roll(den, 32, 1)
            inv = 1.0 / (den + 1e-6)
            pn.append(_cat([a * inv for a in p], 1).astype(BF16))
        o = _dot(_cat(pn), mp[...])
        return [xres[c, r:r + RB, :] + o[r:r + RB] for r in range(0, CH, RB)]

    other[0].wait()

    def first(c, _):
        x_copy(c).wait()
        x = [xio[c, n].astype(F32) for n in range(R1)]
        x = _cat([x[n][u * G:u * G + G] for u in range(NS) for n in range(R1)])
        xres[c] = x
        spec_fwd(c, [x[r:r + RB] for r in range(0, CH, RB)])

    def second(c, _):
        x = attn_out(c)
        xres[c] = _cat(x)
        spec_fwd(c, x)

    def final(c, _):
        x = _cat(attn_out(c))
        for n in range(R1):
            xio[c, n] = _cat([x[(u * R1 + n) * G:(u * R1 + n + 1) * G]
                              for u in range(NS)]).astype(BF16)
        o_copy(c).start()

    def stats(c, _):
        spec_bwd(c)
        attn_stats(c)

    with jax.named_scope("first"):
        lax.fori_loop(0, NC, first, None)
    with jax.named_scope("prepf"):
        other[1].wait()
        other[2].wait()
        prep_filter()
    with jax.named_scope("prepw"):
        other[3].wait()
        other[4].wait()
        prep_weights()

    def layer(l, _):
        with jax.named_scope("mid"):
            spec_mid()
        with jax.named_scope("stats"):
            gacc[...] = jnp.zeros(gacc.shape, F32)
            zacc[...] = jnp.zeros(zacc.shape, F32)
            lax.fori_loop(0, NC, stats, None)
        with jax.named_scope("mix"):
            attn_mix()

        @pl.when(l == 0)
        def _():
            with jax.named_scope("second"):
                lax.fori_loop(0, NC, second, None)

    lax.fori_loop(0, 2, layer, None)
    with jax.named_scope("final"):
        lax.fori_loop(0, NC, final, None)
        for c in range(NC):
            o_copy(c).wait()


@jax.jit
def pallas_interleave_layers__spectral_gfnet__linear_attn_block__prompt_kernel(
    A_x, A_w_r, A_w_i, B_x, B_wqkv, B_wo
):
    del B_x
    vm = pltpu.VMEM
    out = pl.pallas_call(
        _kernel,
        in_specs=[pl.BlockSpec(memory_space=pl.ANY)] * 6,
        out_specs=pl.BlockSpec(memory_space=pl.ANY),
        out_shape=jax.ShapeDtypeStruct((R1, R2, D), BF16),
        scratch_shapes=[
            vm((NC, R1, G * NS, D), BF16),
            vm((NC, CH, D), F32),
            vm((NC, CH, D), BF16),
            vm((16, 128, D), BF16),
            vm((16, 128, D), F32),
            vm((2, DF, S), BF16),
            vm((S // 128, 2, D // 4, 128), I32),
            vm((3, R1 * PITCH, 128), I32),
            vm((D, 3 * D), BF16),
            vm((D, D), BF16),
            vm((D, D), BF16),
            vm((D, D), BF16),
            vm((D, D), F32),
            vm((D, 128), F32),
            vm((NT, D, 128), F32),
            vm((D, D), BF16),
            vm((8, D), F32),
            vm(_MATS.shape, BF16),
            pltpu.SemaphoreType.DMA((NC + 5,)),
        ],
        compiler_params=pltpu.CompilerParams(vmem_limit_bytes=100 * 1024 * 1024),
    )(A_x.reshape(R1, R2, D), A_w_r.T, A_w_i.T, B_wqkv, B_wo, _MATS)
    return out.reshape(1, S, D)
```

```python
import numpy as np
import jax
import jax.numpy as jnp
from jax import lax
import jax.experimental.pallas as pl
import jax.experimental.pallas.tpu as pltpu

S, D, H, DH = 2048, 640, 32, 20
DF = D // 2 + 1
R1, R2 = 32, 64
G = 8
NG = R2 // G
GR = R1 * G
NT = D // 128

_C5 = float(np.sqrt(5.0) / 4.0)
_R5 = float(np.sin(4 * np.pi / 5) / np.sin(2 * np.pi / 5))
_PAIRS = ((0, 0), (1, 1), (2, 1), (1, 2), (2, 2), (3, 3), (4, 3), (3, 4), (4, 4))
_CLASSES = ((0, 5), (4, 6), (1, 9), (2, 8), (3, 7))


def _cmul(re, im, ang):
    c, s = float(np.cos(ang)), float(np.sin(ang))
    if abs(abs(c) - abs(s)) < 1e-12:
        if c * s > 0:
            return (re - im) * c, (re + im) * c
        return (re + im) * c, (im - re) * c
    return re * c - im * s, re * s + im * c


def _cplx_fwd(u, th):
    n = len(u)
    if n == 1:
        return [(th, u[0])]
    h = n // 2
    v = [_cmul(re, im, th / 2) for re, im in u[h:]]
    a = [(p[0] + q[0], p[1] + q[1]) for p, q in zip(u[:h], v)]
    b = [(p[0] - q[0], p[1] - q[1]) for p, q in zip(u[:h], v)]
    return _cplx_fwd(a, th / 2) + _cplx_fwd(b, th / 2 + np.pi)


def _cplx_bwd(g, th):
    n = len(g)
    if n == 1:
        return list(g)
    h = n // 2
    a, b = _cplx_bwd(g[:h], th / 2), _cplx_bwd(g[h:], th / 2 + np.pi)
    lo = [(p[0] + q[0], p[1] + q[1]) for p, q in zip(a, b)]
    hi = [_cmul(p[0] - q[0], p[1] - q[1], -th / 2) for p, q in zip(a, b)]
    return lo + hi


def _real_fwd(x):
    n = len(x)
    if n == 2:
        return [(0.0, (x[0], x[1]))]
    h, q = n // 2, n // 4
    a = [x[j] + x[j + h] for j in range(h)]
    b = [x[j] - x[j + h] for j in range(h)]
    return _real_fwd(a) + _cplx_fwd([(b[j], b[j + q]) for j in range(q)], np.pi / 2)


def _real_bwd(g):
    if len(g) == 1:
        return list(g[0])
    h = len(g) // 2
    a = _real_bwd(g[:h])
    u = _cplx_bwd(g[h:], np.pi / 2)
    b = [p[0] for p in u] + [p[1] for p in u]
    return [p + q for p, q in zip(a, b)] + [p - q for p, q in zip(a, b)]


def _r10_fwd(x, sel, roll, norm=None):
    if sel is not None:
        x = [sel(x[j], x[(j + 2) % 5]) for j in range(5)]
    t1, t2, t3, t4 = x[1] + x[4], x[2] + x[3], x[1] - x[4], x[2] - x[3]
    t5 = t1 + t2
    y0, m1, m2 = x[0] + t5, x[0] - t5 * 0.25, (t1 - t2) * _C5
    out = []
    for re, im in ((m1 + m2, t3 + t4 * _R5), (m1 - m2, t3 * _R5 - t4)):
        if sel is None:
            out += [re, im]
        else:
            a, b = sel(re, im), roll(sel(im, re))
            out += [a + b, a - b]
    if norm is None:
        return [y0] + out
    y0, scale = norm(y0, m1, m2, t3, t4)
    return [a * scale for a in [y0] + out]


def _r10_bwd(g, sel, roll):
    re, im = [], []
    for u, v in ((g[1], g[2]), (g[3], g[4])):
        if sel is not None:
            a, b = u + v, roll(u - v)
            u, v = sel(a, b), sel(b, a)
        re.append(u)
        im.append(v)
    m1, e = re[0] + re[1], (re[0] - re[1]) * _C5
    t5 = g[0] - m1 * 0.25
    t1, t2 = t5 + e, t5 - e
    t3, t4 = im[0] + im[1] * _R5, im[0] * _R5 - im[1]
    x = [g[0] + m1, t1 + t3, t2 + t4, t2 - t4, t1 - t3]
    return x if sel is None else [sel(x[j], x[(j + 3) % 5]) for j in range(5)]


def _build_constants():
    lane = np.arange(128)
    grp = [np.concatenate([c + 10 * np.arange(32) for c in cls]) for cls in _CLASSES]
    d = np.arange(D)[:, None]
    cols = []
    for g, kd in enumerate(grp):
        c, s = np.cos(2 * np.pi * d * kd / D), np.sin(2 * np.pi * d * kd / D)
        if g == 0:
            s[:, 0] = np.cos(np.pi * d[:, 0])
        cols.append(np.concatenate([s, c] if g in (2, 4) else [c, s], axis=1))
    eye = np.eye(D)
    net = np.concatenate(_r10_fwd(
        [eye[:, 128 * j:128 * j + 128] for j in range(NT)],
        lambda a, b: np.where(lane < 64, a, b), lambda a: np.roll(a, 64, axis=1)), axis=1)
    bd = np.linalg.solve(net, np.concatenate(cols, axis=1))
    fd = np.stack([bd[128 * j:128 * j + 128, 128 * j:128 * j + 128] for j in range(NT)])
    assert abs(np.abs(bd).sum() - np.abs(fd).sum()) < 1e-6
    dmat = np.concatenate([fd, fd.transpose(0, 2, 1) / D])

    cs = [cols[0]] + [np.concatenate(p, axis=1) for j in (1, 3) for p in (
        (cols[j][:, :64], cols[j + 1][:, 64:]), (cols[j][:, 64:], cols[j + 1][:, :64]))]
    net = np.concatenate(_r10_fwd(
        [eye[:, 128 * j:128 * j + 128] for j in range(NT)], None, None), axis=1)
    bd = np.linalg.solve(net, np.concatenate(cs, axis=1))
    f5, i5 = (np.stack([m[128 * i:128 * i + 128, 128 * j:128 * j + 128] for i, j in _PAIRS])
              for m in (bd, bd.T / D))
    assert abs(np.abs(bd).sum() - np.abs(f5).sum()) < 1e-6

    leaves = [int(round(th * R1 / (2 * np.pi))) for th, _ in _real_fwd(list(np.eye(R1)))]
    k1 = [min(m, R1 - m) for m in leaves]
    pos = np.arange(128)
    part, n2 = (pos // G) % 2, (pos // (2 * G)) * G + pos % G
    packed = (pos // (2 * G)) * 2 * G + (pos % 2) * G + (pos % (2 * G)) // 2
    fs = []
    for m, kk in zip(leaves, k1):
        ks = (16 * np.arange(R2) if m == 0 else kk + R1 * np.arange(R2))[:, None]
        if m == 0:
            ph = 2 * np.pi * ks * (n2 + R2 * part) / S
            c, s = np.cos(ph), np.sin(ph)
            s[0] = np.cos(np.pi * n2)
        else:
            sg = 1.0 if m == kk else -1.0
            ph = 2 * np.pi * ks * n2 / S
            c = np.where(part == 0, np.cos(ph), -sg * np.sin(ph))
            s = np.where(part == 0, np.sin(ph), sg * np.cos(ph))
        fs.append(np.concatenate([c, s]))
    fs = np.stack(fs)[:, part * R2 + n2]
    smat = np.concatenate([fs[:, :, packed], fs.transpose(0, 2, 1) * (2.0 / S)])

    have = np.concatenate([R1 * np.arange(R2), 16 + R1 * (R2 - 1 - np.arange(R2))])
    want = np.concatenate([16 * np.arange(R2), S // 2 + 16 * ((R2 - np.arange(R2)) % R2)])
    p0 = (want[:, None] == have[None, :]).astype(np.float64)

    mats = np.concatenate([f5, smat, p0[None], i5, dmat[NT:], dmat[:NT]]).astype(jnp.bfloat16)
    mats = mats.view(np.uint16).astype(np.uint32)
    return (mats[:, 0::2] | (mats[:, 1::2] << 16)).view(np.int32), k1


_MATS, _K1 = _build_constants()
_F5, _SF, _SI, _P0, _I5, _DI, _DF, _NM = 0, 9, 25, 41, 42, 51, 56, 61
from functools import partial

F32, BF16, I32 = jnp.float32, jnp.bfloat16, jnp.int32
PITCH = 68
FB = 16
MB = 128
LAG = 2
PRE = 0
F5 = 6
B5 = 1
SK, SG, SQ, SO = 1, 1, 1, 1
HR = GR // 2
QL = 1
SKL = 0
DB = 128
nop = lambda: None
KB = 160
XB = 256
AHEAD = 3
_MCUT = (0, _SF, _SI, _I5, _DF, _NM)
NW = 4
WL = S // NW
_HI = np.int32(-65536)

RB = 16
_WIN = ((0, 144), (112, 272), (240, 400), (368, 528), (496, 640))


def _dot(a, b):
    return jnp.dot(a.astype(BF16), b.astype(BF16), preferred_element_type=F32)


def _dot_nt(a, b):
    return lax.dot_general(a.astype(BF16), b.astype(BF16), (((1,), (1,)), ((), ())), preferred_element_type=F32)


def _sel(a, b):
    return jnp.where(lax.broadcasted_iota(I32, a.shape, 1) < 64, a, b)


def _roll(a):
    return pltpu.roll(a, 64, 1)


def _tiles(a):
    return [a[:, 128 * j:128 * j + 128] for j in range(a.shape[1] // 128)]


def _cat(a, axis=0):
    return a[0] if len(a) == 1 else jnp.concatenate(a, axis=axis)


def _split(a):
    return [_cat([a[r:r + G] for r in range(o, a.shape[0], 2 * G)]) for o in (0, G)]


def _merge(a, b):
    return _cat([x[r:r + G] for r in range(0, a.shape[0], G) for x in (a, b)])


def _quads(a, h, w):
    return a[:h, :w], a[:h, w:2 * w], a[h:2 * h, :w], a[h:2 * h, w:2 * w]


def _terms_a(a11, a12, a21, a22):
    return a11 + a22, a22 - a21, a11, a22, a11 - a12, a21 + a11, a12 + a22


def _terms_w(w11, w12, w21, w22):
    return w11 + w22, w11, w12 + w22, w21 + w11, w22, w12 - w11, w21 - w22


_USE = (((0, 1), (3, 1)), ((2, -1), (3, -1)), ((1, 1), (3, -1)), ((0, -1), (2, 1)),
        ((0, -1), (1, -1)), ((3, 1),), ((0, 1),))
_ORD = tuple(int(c) for c in '6034215')


def _combine(c, p):
    c = list(c)
    for i in reversed(_ORD):
        for k, sg in _USE[i]:
            c[k] = c[k] + p[i] if sg > 0 else c[k] - p[i]
    return c


def _words(a):
    return pltpu.bitcast(a, I32)


def _phi(t):
    return jnp.where(t > 0, t + 1.0, jnp.exp(t)) + 1e-6


def _ln(x):
    mean = jnp.sum(x[0] + x[1] + x[2] + x[3] + x[4], axis=1, keepdims=True) * (1.0 / D)
    x = [a - mean for a in x]
    sq = x[0] * x[0] + x[1] * x[1] + x[2] * x[2] + x[3] * x[3] + x[4] * x[4]
    r = lax.rsqrt(jnp.sum(sq, axis=1, keepdims=True) * (1.0 / D) + 1e-5)
    return [a * r for a in x]


def _lane_sum(a):
    return jnp.sum(a, axis=1, keepdims=True)


def _lane_sum_mxu(a):
    hi = pltpu.bitcast(_words(a) & _HI, F32)
    return _dot(_cat([hi, a - hi], 1), jnp.ones((256, 128), BF16))


def _ln_r5(y0, m1, m2, t3, t4, lane_sum=_lane_sum):
    y0 = y0 - lane_sum(y0) * (1.0 / 128)
    sq = (m1 * m1 + m2 * m2) * 4.0 + (t3 * t3 + t4 * t4) * 2.5 + y0 * y0
    return y0, lax.rsqrt(lane_sum(sq) * (0.2 / D) + 1e-5)


def _bf(a):
    return pltpu.bitcast(a, BF16)


def _run(*gens):
    gens = [list(g) for g in gens]
    order = sorted(((i + 0.5) / len(g), k, i) for k, g in enumerate(gens) for i in range(len(g)))
    for _, k, i in order:
        gens[k][i]()


def _zip(a, b):
    n = len(b) // max(len(a), 1)
    return [f for i, p in enumerate(a) for f in [p] + b[i * n:i * n + n]]


def _ds(start, size, align=None):
    if isinstance(start, int):
        return pl.ds(start, size)
    return pl.ds(pl.multiple_of(start, align or size), size)


def _kernel(x_hbm, wr_hbm, wi_hbm, wqkv_hbm, wo_hbm, mats_hbm, o_hbm,
            xio, ybuf, z0, wraw, wtmp, wbuf, wqkv, wo, wqt, zacc, macc, mats, sems, bsem):

    def x_copy(c):
        return pltpu.make_async_copy(x_hbm.at[:, _ds(G * c, G), :], xio.at[c], sems.at[c & 3])

    def o_copy(c, h):
        n1 = pl.ds(h * (R1 // 2), R1 // 2)
        return pltpu.make_async_copy(xio.at[c, n1], o_hbm.at[n1, _ds(G * c, G), :], sems.at[0])

    def w_copy(i, c):
        return pltpu.make_async_copy(
            (wr_hbm, wi_hbm)[i].at[:, _ds(WL * c, WL)], wraw.at[i, c], sems.at[6 + c % 4])

    def m_copy(i):
        lo, hi = _MCUT[i], _MCUT[i + 1]
        return pltpu.make_async_copy(mats_hbm.at[lo:hi], mats.at[lo:hi], sems.at[4 + i % 2])

    def a_copy(k, i):
        rs = pl.ds(128 * i, 128)
        if k == 3:
            return pltpu.make_async_copy(wo_hbm.at[rs], wo.at[rs], sems.at[2])
        return pltpu.make_async_copy(
            wqkv_hbm.at[rs, pl.ds(D * k, D)], wqkv.at[k, rs], sems.at[1 if k == 1 else 2])

    mat = lambda i: _bf(mats[i])
    st = {}

    def fwd_rows(g, r, x):
        st["t", g, r] = _r10_fwd(_tiles(x), _sel if g < F5 else None, _roll, _ln_r5)

    def d5(t, base, j):
        ks = [k for k, p in enumerate(_PAIRS) if p[1] == j]
        return _dot(_cat([t(_PAIRS[k][0]) for k in ks], 1),
                    _cat([mat(base + k) for k in ks]))

    def load_x(g, r, n):
        return _cat([xio[g, i].astype(F32) for i in range(r // G, (r + n) // G)])

    def d_fwd(g):
        def step(j):
            t = lambda i: _cat([st["t", g, r][i] for r in range(0, GR, RB)])
            st["y", g, j] = _dot(t(j).astype(BF16), mat(_DF + j)) if g < F5 else d5(t, _F5, j)
        return [partial(step, j) for j in range(NT)]

    def s_fwd(g, row=None):
        def put(s, j, w):
            if row is None:
                st["z", s, g, j] = w
            else:
                z0[s, _ds(row, G), 128 * j:128 * j + 128] = w

        def step(j):
            y = st["y", g, j]
            v = _real_fwd([y[n * G:n * G + G, :] for n in range(R1)])
            w = [pltpu.pack_elementwise(list(p), packed_dtype=BF16).astype(I32) for _, p in v]
            st["w", g, j] = w
            for s in range(16):
                if j == 0 or g >= F5:
                    put(s, j, w[s])
                elif j % 2 == 0:
                    a, b = st["w", g, j - 1][s], w[s]
                    put(s, j - 1, _sel(a, b))
                    put(s, j, _roll(_sel(b, a)))
        return [partial(step, j) for j in range(NT)]

    def s_bwd(g):
        def step(j):
            r0 = 2 * G * g
            w = _cat(_real_bwd([(st["zi", s, j][r0:r0 + G], st["zi", s, j][r0 + G:r0 + 2 * G])
                                for s in range(16)]))
            st["u", g, j] = w
            if j and j % 2 == 0 and g >= B5:
                a, b = st["u", g, j - 1], _roll(w)
                st["u", g, j - 1], st["u", g, j] = _sel(a, b), _sel(b, a)
        return [partial(step, j) for j in range(NT)]

    def d_bwd(g):
        def step(r, j):
            t = lambda i: st["u", g, i][r:r + DB]
            st["v", g, j] = _dot(t(j), mat(_DI + j)) if g >= B5 else d5(t, _I5, j)
            if j == NT - 1:
                _run(bwd_rows(g)[r // RB:(r + DB) // RB])
        return [partial(step, r, j) for r in range(0, GR, DB) for j in range(NT)]

    def bwd_rows(g):
        def step(r):
            d = _r10_bwd([st["v", g, j][r % DB:r % DB + RB] for j in range(NT)],
                         _sel if g >= B5 else None, _roll)
            x = st["res", g, r] if ("res", g, r) in st else load_x(g, r, RB)
            x = [a + b for a, b in zip(_tiles(x), d)]
            st["res", g, r] = _cat(x, 1)
            st["xn", g, r] = _cat(_ln(x), 1)
        return [partial(step, r) for r in range(0, GR, RB)]

    def prep_filter(c, t):
        ls = slice(128 * t, 128 * t + 128)

        def merge():
            a, b = _words(wraw[0, c, 0:D // 2, ls]), _words(wraw[1, c, 0:D // 2, ls])
            wtmp[c, t, 0] = (a << 16) | (b & 0xFFFF)
            wtmp[c, t, 1] = (a & _HI) | lax.shift_right_logical(b, 16)

        def step(j):
            cls = lambda k: wtmp[c, t, k % 2, pl.ds(k // 2, 32, stride=5), :]
            if j == 0:
                last = _words(wraw[0, c, D // 2:DF, ls].astype(F32)) | lax.shift_right_logical(
                    _words(wraw[1, c, D // 2:DF, ls].astype(F32)), 16)
                c0, c5 = cls(0), cls(5)
                src = [c0, c5, jnp.where(lax.broadcasted_iota(I32, c0.shape, 0) == 0, last, c0), c5]
            else:
                src = [cls(k) for k in _CLASSES[2 * j - 1] + _CLASSES[2 * j]]
            w = _cat(src).T
            for i in range(16):
                k2, k1 = (WL // R1) * c + 4 * t + i // 4, 8 * (i % 4)
                pos = k2 if k1 < 16 else R2 - 1 - k2
                wbuf[j, pl.ds(k1 * PITCH + pos, 8, stride=PITCH), :] = w[8 * i:8 * i + 8]
        return [merge] + [partial(step, j) for j in range(3)]

    def prep_filter_end():
        for j in range(3):
            w = _cat([wbuf[j, 0:R2, :], wbuf[j, 16 * PITCH:16 * PITCH + R2, :]])
            re = _dot(mat(_P0), pltpu.bitcast(w & _HI, F32).astype(BF16))
            im = _dot(mat(_P0), pltpu.bitcast(w << 16, F32).astype(BF16))
            w = _words(re) | lax.shift_right_logical(_words(im), 16)
            wbuf[j, 0:R2, :] = w[:R2]
            wbuf[j, 16 * PITCH:16 * PITCH + R2, :] = w[R2:]

    def prep_wq(i):
        r0 = (0, 256, 384)[i]
        wqt[i] = _words(wqkv[0, r0:r0 + 256, :]).T
        w = _cat([wqt[i, pl.ds(d, H, stride=DH), :] for d in range(DH)]).T
        st["wq", i] = _bf(w[64:] if i == 2 else w)
        if i == 2:
            w = _cat([st["wq", k] for k in range(3)])
            st["wqs"] = w, _terms_w(*_quads(w.astype(F32), 256, 256))

    def prep_wk(j):
        st["wk", j] = wqkv[1, :, 128 * j:128 * j + 128].astype(F32).T
        if j == NT - 1:
            w = _cat([st["wk", i] for i in range(NT)])
            w11, w21, w12, w22 = _quads(w, D // 2, 256)
            st["wkt"], st["wks"] = w, _terms_w(w11, w12, w21, w22)

    def mid_fwd(s, tiles):
        for j in tiles:
            if ("z", s, 0, j) in st:
                a = _cat([st["z", s, g, j] for g in range(NG)])
            else:
                a = z0[s, :, 128 * j:128 * j + 128]
            st["x", s, j] = _dot(mat(_SF + s), _bf(a))

    def mid_filter(s, tiles):
        k1 = _K1[s]
        p1, p2 = k1 * PITCH, (R1 - k1 if k1 else 16) * PITCH
        if k1:
            m = lambda a: a
        else:
            row0 = lax.broadcasted_iota(I32, (R2, 128), 0) == 0
            m = lambda a: jnp.where(row0, 0.0, a)

        def coef(j, p):
            w = wbuf[j, p:p + R2, :]
            return pltpu.bitcast(w & _HI, F32), pltpu.bitcast(w << 16, F32)

        for j in tiles:
            if j == 0:
                lane = lax.broadcasted_iota(I32, (R2, 128), 1)
                edge = (lane & 63) == 0
                sgn = jnp.where(lane < 64, -1.0, 1.0)
                s0 = jnp.where(edge, 0.0, sgn)
                tc, ts = _split(st["x", s, 0])
                a, b = _sel(tc, ts), _sel(ts, tc)
                re, im = a + m(_roll(a) * s0), m(b) - _roll(b) * s0
                (a1, b1), (a2, b2) = coef(0, p1), coef(0, p2)
                cr = jnp.where(edge, (a1 + a2) * 0.5, _sel(a1, a2))
                ci = jnp.where(edge, (b2 - b1) * (sgn * 0.5), _sel(b1, b2))
                re, im = cr * re + ci * im, cr * im - ci * re
                an, bn = re - m(_roll(re) * s0), m(im) + _roll(im) * s0
                if not k1:
                    an = jnp.where(row0 & edge, a * _sel(a1, a2) * 0.5, an)
                    bn = jnp.where(row0 & edge, b * _sel(a2, a1) * 0.5, bn)
                st["f", s, 0] = _merge(_sel(an, bn), _sel(bn, an))
            elif j % 2:
                cc, sc = _split(st["x", s, j])
                cs, ss = _split(st["x", s, j + 1])
                r1, n1, r2, n2 = cc - m(ss), cs + m(sc), m(cc) + ss, m(cs) - sc
                (a1, b1), (a2, b2) = coef((j + 1) // 2, p1), coef((j + 1) // 2, p2)
                r1, n1 = a1 * r1 + b1 * n1, a1 * n1 - b1 * r1
                r2, n2 = a2 * r2 + b2 * n2, a2 * n2 - b2 * r2
                st["f", s, j] = _merge(r1 + m(r2), m(n1) - n2)
                st["f", s, j + 1] = _merge(n1 + m(n2), r2 - m(r1))

    def mid_bwd(s, tiles):
        for j in tiles:
            st["zi", s, j] = _dot(mat(_SI + s), st["f", s, j].astype(BF16))

    def half(g, h):
        if g < SKL or g >= 0:
            return range(h * HR, h * HR + HR, RB)
        return range(h * RB, GR, 2 * RB)

    def terms(name, g):
        if (name, g) not in st:
            a = _cat([st[name, g, r] for h in (0, 1) for r in half(g, h)])
            st[name, g] = a, _terms_a(*_quads(a, HR, 256))
        return st[name, g]

    def proj(name, g, w, out, fast, then):
        def put(o, y):
            for i, r in enumerate(half(g, o)):
                st[out, g, r] = y[i * RB:i * RB + RB]

        def plain(h):
            put(h, _dot(terms(name, g)[0][h * HR:h * HR + HR], st[w][0]))
            _run([then[r // RB] for r in half(g, h)])

        def side():
            st["e", out] = _dot(terms(name, g)[0], st[w][0][:, 512:])

        def edge():
            c = _dot(terms(name, g)[0][:, 512:], st[w][0][512:, :512])
            c = _combine(_quads(c, HR, 256), [st["c", out, i] for i in range(7)])
            put(0, _cat([c[0], c[1], st["e", out][:HR]], 1))
            put(1, _cat([c[2], c[3], st["e", out][HR:]], 1))
            _run(then)

        def step(i):
            st["c", out, i] = _dot(terms(name, g)[1][i], st[w][1][i])
        if not fast:
            return [partial(plain, h) for h in (0, 1)]
        return [side] + [partial(step, i) for i in _ORD] + [edge]

    def k_mm(g):
        def edge(r):
            if g >= SKL:
                a = terms("xn", g)[0][:, 512:]
                e = [_dot_nt(st["wkt"][o:o + KB, 512:], a) for o in (r, D // 2 + r)]
                c = _combine([e[0][:, :HR], e[1][:, :HR], e[0][:, HR:], e[1][:, HR:]],
                             [st["ck", i] for i in range(7)])
            else:
                c = [st["k0"][o:o + KB] for o in (r, D // 2 + r)] + [
                    _dot_nt(st["wkt"][o:o + KB], terms("xn", g)[0][HR:]) for o in (r, D // 2 + r)]
            c = [_phi(a) for a in c]
            for o, zs in ((r, c[0] + c[2]), (D // 2 + r, c[1] + c[3])):
                zacc[o:o + KB, :] = zacc[o:o + KB, :] + zs if g else zs
            st["pk", g, r] = ([_cat(c[i::2], 1) for i in (0, 1)],
                              _terms_a(c[0], c[2], c[1], c[3]))

        def step(r, i):
            st["ck", i] = _dot_nt(st["wks"][i][r:r + KB], terms("xn", g)[1][i])

        def plain():
            st["k0"] = _dot_nt(st["wkt"], terms("xn", g)[0][:HR])
        if g < SKL:
            return [plain] + [partial(edge, r) for r in range(0, D // 2, KB)]
        return [f for r in range(0, D // 2, KB) for f in [
            partial(step, r, i) for i in _ORD] + [partial(edge, r)]]

    def g_mm(g):
        n = abs(SG or 1)
        gs = list(range(g - g % n, g - g % n + n))

        def add(key, a, x):
            a = _dot(_cat(a, 1), _cat(x))
            st[key] = st[key] + a if gs[0] else a

        def edge(r, i):
            add(("g", D // 2 * i + r), [st["pk", k, r][0][i] for k in gs],
                [terms("xn", k)[0][:, 512 if SG > 0 else 0:] for k in gs])

        def step(r, i):
            add(("gs", r, i), [st["pk", k, r][1][i] for k in gs],
                [terms("xn", k)[1][(0, 2, 6, 5, 3, 4, 1)[i]] for k in gs])
        fs = [f for r in range(0, D // 2, KB) for f in [partial(edge, r, 0), partial(edge, r, 1)]
              + [partial(step, r, i) for i in range(7 if SG > 0 else 0)]]
        return fs[len(fs) * (g % n) // n:len(fs) * (g % n + 1) // n]

    def mix_z():
        zp = _cat([zacc[pl.ds(d, H, stride=DH), :] for d in range(DH)])
        st["zrow"] = jnp.broadcast_to(jnp.sum(zp.T, axis=0, keepdims=True), (RB, D))

    def mix_kv():
        gm = _cat([st["g", r] for r in range(0, D, KB)])
        if SG > 0:
            m1, m2, n3, n4, m5, n6, n7 = (
                _cat([st["gs", r, i] for r in range(0, D // 2, KB)]) for i in range(7))
            gm = _cat([_cat([m1 - n4 - m5 - n7, n4 - m2]),
                       _cat([n3 - m5, m1 - m2 - n3 - n6]), gm], 1)
        for j, (r0, r1) in enumerate(_WIN):
            kv = _dot(gm[r0:r1].astype(BF16),
                      wqkv[2, :, 128 * j:128 * j + 128])
            hr = ((lax.broadcasted_iota(I32, kv.shape, 0) + r0) * 3277) >> 16
            hc = ((lax.broadcasted_iota(I32, kv.shape, 1) + 128 * j) * 3277) >> 16
            st["kv", j] = jnp.where(hr == hc, kv, 0.0).astype(BF16)

    def mix_m():
        done = 0
        for j, (r0, r1) in enumerate(_WIN):
            m = _dot(st["kv", j], wo[128 * j:128 * j + 128, :])
            for t, a in enumerate(_tiles(m)):
                if done > r0:
                    macc[t, r0:done, :] += a[:done - r0]
                macc[t, done:r1, :] = a[done - r0:]
            done = r1
        w = _cat([_cat([macc[t, pl.ds(d, H, stride=DH), :] for d in range(DH)])
                  for t in range(NT)], 1)
        st["m"] = w, _terms_w(*_quads(w, 256, 256))

    def q_mm(g):
        return proj("xn", g, "wqs", "q", SQ, q_act(g))

    def q_act(g):
        def step(r):
            zt = _tiles(st["zrow"])
            p = _tiles(_phi(st["q", g, r]))
            den = p[0] * zt[0] + p[1] * zt[1] + p[2] * zt[2] + p[3] * zt[3] + p[4] * zt[4]
            den = den + _roll(den)
            den = den + pltpu.roll(den, 32, 1)
            inv = 1.0 / (den + 1e-6)
            st["p", g, r] = _cat([a * inv for a in p], 1)
        return [partial(step, r) for r in range(0, GR, RB)]

    def o_mm(g, last):
        return proj("p", g, "m", "o", g < (8 if last else 0), o_rows(g, last))

    def o_rows(g, last):
        def step(r):
            x = st["res", g, r] + st["o", g, r]
            if last:
                for i in range(0, RB, G):
                    xio[g, (r + i) // G] = x[i:i + G].astype(BF16)
                st["n", g, r // HR] = st.get(("n", g, r // HR), 0) + RB
                if st["n", g, r // HR] == HR:
                    o_copy(g, r // HR).start()
            else:
                st["res", g, r] = x
                fwd_rows(g, r, x)
        return [partial(step, r) for r in range(0, GR, RB)]

    def fence():
        if 1 == 1:
            pl.semaphore_signal(bsem)
            pl.semaphore_wait(bsem)
        elif 1 == 2:
            pl.delay(1)
        else:
            def body(i, _):
                wqt[0, pl.ds(i, 1), :] = jnp.zeros((1, 128), I32)
            lax.fori_loop(0, 2, body, None)

    def _scope(n):
        if n[0] + n[-1] in 's0,s1,o1':
            fence()
        return jax.named_scope(n)

    def at(f, g, *a):
        return f(g, *a) if 0 <= g < NG else []

    def rows(c):
        def step(r):
            t = _r10_fwd(_tiles(load_x(c, r, XB)), None, None,
                         partial(_ln_r5, lane_sum=_lane_sum_mxu if 0 else _lane_sum))
            for j in range(NT):
                ybuf[j, r:r + XB, :] = t[j]
        return [partial(step, r) for r in range(0, GR, XB)]

    def cols(c):
        for j in range(NT):
            st["y", NG, j] = d5(lambda i: ybuf[i], _F5, j)
        return s_fwd(NG, G * c)

    def filt(c):
        w_copy(0, c).wait()
        w_copy(1, c).wait()
        return sum([prep_filter(c, t) for t in range(WL // 128)], [])

    def w_start(c):
        w_copy(0, c).start()
        w_copy(1, c).start()

    W0 = [int(c) for c in '4567']

    def first(c, _):
        x_copy(c).wait()
        when = (lambda p: lambda f: f() if p else None) if isinstance(c, int) else pl.when
        when(c + AHEAD < NG)(lambda: x_copy(c + AHEAD).start())
        when(c == 5)(lambda: m_copy(1).start())
        for i, k in enumerate(W0):
            when(c == k)(partial(w_start, i))
        _run(rows(c), cols(c - 1))

    x_copy(0).start()
    m_copy(0).start()
    x_copy(1).start()
    with _scope("first"):
        x_copy(0).wait()
        for c in range(2, AHEAD + 1):
            x_copy(c).start()
        _run(rows(0))
        m_copy(0).wait()
        if 0:
            for c in range(1, NG):
                first(c, None)
        else:
            lax.fori_loop(1, NG, first, None)

    order = list(range(1, 16)) + [0]
    for layer in range(2):
        for g in range(NG):
            st.pop(("xn", g), None)
            st.pop(("p", g), None)
        with _scope("mid%d" % layer):
            if layer == 0:
                m_copy(1).wait()
                for c in range(NW):
                    pf = filt(c)
                    k = c + len(W0) - NW
                    if k < 0:
                        w_start(NW + k)
                    if k == 0:
                        m_copy(2).start()
                    if c == NW - 1:
                        m_copy(3).start()
                        for j in range(NT):
                            a_copy(1, j).start()
                    n = 16 // (NW - 1) + 1
                    _run(pf, [partial(mid_fwd, s, range(NT)) for s in order[n * c - n:n * c]]
                         if c else cols(NG - 1))
                m_copy(2).wait()
                if 9 == 0:
                    m_copy(3).wait()
                    for j in range(NT):
                        a_copy(1, j).wait()
                    o_copy(0, 0).start()
                    o_copy(0, 0).wait()
                    return
            for i in range(16 + LAG):
                if layer == 0 and i == 2:
                    prep_filter_end()
                if layer == 0 and i == 12:
                    m_copy(3).wait()
                    for j in range(NT):
                        a_copy(1, j).wait()
                    m_copy(4).start()
                    for j in range(NT):
                        prep_wk(j)
                if layer and i < 16:
                    mid_fwd(order[i], range(NT))
                if i >= LAG:
                    mid_bwd(order[i - LAG], range(NT))
                if i < 16:
                    mid_filter(order[i], range(NT))
        with _scope("stats%d" % layer):
            for g in range(NG + 1 + abs(SG or 1)):
                if layer == 0:
                    if 1 <= g <= NT:
                        wqkv[0, 128 * g - 128:128 * g - 112, :128] = st["xn", g - 1, 0][:16, :128].astype(BF16)
                        for k in (0, 2, 3):
                            a_copy(k, g - 1).start()
                    if g == NT + 2:
                        m_copy(4).wait()
                        for k in (0, 2, 3):
                            for j in range(NT):
                                a_copy(k, j).wait()
                    if NT + 2 <= g < NT + 5:
                        prep_wq(g - NT - 2)
                _run(at(s_bwd, g))
                gm, km, dm = at(g_mm, g - 1 - abs(SG or 1)), at(k_mm, g - 1), at(d_bwd, g)
                dm = [nop] * (0 if g == 1 else 0) + dm + [nop] * (len(dm) * 2 // 4)
                if 1:
                    _run(dm, gm, km)
                else:
                    _run(dm, gm + km)
        with _scope("out%d" % layer):
            mix_z()
            _run(q_mm(0))
            mix_kv()
            if QL > 1:
                _run(q_mm(1))
            mix_m()
            for g in range(NG + 1):
                qm, om = at(q_mm, g + QL), at(o_mm, g, layer == 1)
                dm = _zip(at(d_fwd, g - 1), at(s_fwd, g - 1)) if layer == 0 else []
                dm = [nop] * (len(dm) * 4 // 4) + dm
                if 0 and g:
                    _run(qm + [nop] * 0, [nop] * 0 + om, dm)
                else:
                    _run(qm + om, dm)
    for c in range(NG):
        o_copy(c, 0).wait()
        o_copy(c, 1).wait()


@jax.jit
def pallas_interleave_layers__spectral_gfnet__linear_attn_block__prompt_kernel(
    A_x, A_w_r, A_w_i, B_x, B_wqkv, B_wo
):
    del B_x
    vm = pltpu.VMEM
    out = pl.pallas_call(
        _kernel,
        in_specs=[pl.BlockSpec(memory_space=pl.ANY)] * 6,
        out_specs=pl.BlockSpec(memory_space=pl.ANY),
        out_shape=jax.ShapeDtypeStruct((R1, R2, D), BF16),
        scratch_shapes=[
            vm((NG, R1, G, D), BF16),
            vm((NT, GR, 128), F32),
            vm((16, R2, D), I32),
            vm((2, S // WL, DF, WL), BF16),
            vm((NW, WL // 128, 2, D // 4, 128), I32),
            vm((3, R1 * PITCH, 128), I32),
            vm((3, D, D), BF16),
            vm((D, D), BF16),
            vm((3, D, 128), I32),
            vm((D, 128), F32),
            vm((NT, D, 128), F32),
            vm(_MATS.shape, I32),
            pltpu.SemaphoreType.DMA((10,)),
            pltpu.SemaphoreType.REGULAR,
        ],
        compiler_params=pltpu.CompilerParams(vmem_limit_bytes=100 * 1024 * 1024, disable_bounds_checks=bool(1), flags={k: True for k in ('XLA_TPU_FORCE_LP_LLO_SCHEDULER' if 0 else '').split(',') if k} or None),
    )(A_x.reshape(R1, R2, D), A_w_r.T, A_w_i.T, B_wqkv, B_wo, _MATS)
    return out.reshape(1, S, D)
```

```python
from functools import partial

import numpy as np
import jax
import jax.numpy as jnp
from jax import lax
import jax.experimental.pallas as pl
import jax.experimental.pallas.tpu as pltpu

S, D, H, DH = 2048, 640, 32, 20
DF = D // 2 + 1
R1, R2 = 32, 64
G = 8
NG = R2 // G
GR = R1 * G
NT = D // 128

_C5 = float(np.sqrt(5.0) / 4.0)
_R5 = float(np.sin(4 * np.pi / 5) / np.sin(2 * np.pi / 5))
_PAIRS = ((0, 0), (1, 1), (2, 1), (1, 2), (2, 2), (3, 3), (4, 3), (3, 4), (4, 4))
_CLASSES = ((0, 5), (4, 6), (1, 9), (2, 8), (3, 7))


def _cmul(re, im, ang):
    c, s = float(np.cos(ang)), float(np.sin(ang))
    if abs(abs(c) - abs(s)) < 1e-12:
        if c * s > 0:
            return (re - im) * c, (re + im) * c
        return (re + im) * c, (im - re) * c
    return re * c - im * s, re * s + im * c


def _cadd(p, q):
    return p[0] + q[0], p[1] + q[1]


def _csub(p, q):
    return p[0] - q[0], p[1] - q[1]


def _cplx_fwd(u, th):
    n = len(u)
    if n == 1:
        return [(th, u[0])]
    if n == 4:
        v1, v2, v3 = (_cmul(*u[k], k * th / 4) for k in (1, 2, 3))
        a, b, c, d = _cadd(u[0], v2), _csub(u[0], v2), _cadd(v1, v3), _csub(v1, v3)
        out = _cadd(a, c), _csub(a, c), (b[0] - d[1], b[1] + d[0]), (b[0] + d[1], b[1] - d[0])
        return [(th / 4 + k * np.pi / 2, o) for k, o in zip((0, 2, 1, 3), out)]
    h = n // 2
    v = [_cmul(re, im, th / 2) for re, im in u[h:]]
    a = [_cadd(p, q) for p, q in zip(u[:h], v)]
    b = [_csub(p, q) for p, q in zip(u[:h], v)]
    return _cplx_fwd(a, th / 2) + _cplx_fwd(b, th / 2 + np.pi)


def _cplx_bwd(g, th):
    n = len(g)
    if n == 1:
        return list(g)
    if n == 4:
        a, c, b = _cadd(g[0], g[1]), _csub(g[0], g[1]), _cadd(g[2], g[3])
        d = (g[2][1] - g[3][1], g[3][0] - g[2][0])
        v = _cadd(c, d), _csub(a, b), _csub(c, d)
        return [_cadd(a, b)] + [_cmul(*v[k - 1], -k * th / 4) for k in (1, 2, 3)]
    h = n // 2
    a, b = _cplx_bwd(g[:h], th / 2), _cplx_bwd(g[h:], th / 2 + np.pi)
    return [_cadd(p, q) for p, q in zip(a, b)] + [
        _cmul(*_csub(p, q), -th / 2) for p, q in zip(a, b)]


def _real_fwd(x):
    n = len(x)
    if n == 2:
        return [(0.0, (x[0], x[1]))]
    h, q = n // 2, n // 4
    a = [x[j] + x[j + h] for j in range(h)]
    b = [x[j] - x[j + h] for j in range(h)]
    return _real_fwd(a) + _cplx_fwd([(b[j], b[j + q]) for j in range(q)], np.pi / 2)


def _real_bwd(g):
    if len(g) == 1:
        return list(g[0])
    h = len(g) // 2
    a = _real_bwd(g[:h])
    u = _cplx_bwd(g[h:], np.pi / 2)
    b = [p[0] for p in u] + [p[1] for p in u]
    return [p + q for p, q in zip(a, b)] + [p - q for p, q in zip(a, b)]


def _r10_fwd(x, sel, roll, norm=None):
    if sel is not None:
        x = [sel(x[j], x[(j + 2) % 5]) for j in range(5)]
    t1, t2, t3, t4 = x[1] + x[4], x[2] + x[3], x[1] - x[4], x[2] - x[3]
    t5 = t1 + t2
    y0, m1, m2 = x[0] + t5, x[0] - t5 * 0.25, (t1 - t2) * _C5
    out = []
    for re, im in ((m1 + m2, t3 + t4 * _R5), (m1 - m2, t3 * _R5 - t4)):
        if sel is None:
            out += [re, im]
        else:
            a, b = sel(re, im), roll(sel(im, re))
            out += [a + b, a - b]
    if norm is None:
        return [y0] + out
    y0, scale = norm(y0, m1, m2, t3, t4)
    return [a * scale for a in [y0] + out]


def _r10_bwd(g, sel, roll):
    re, im = [], []
    for u, v in ((g[1], g[2]), (g[3], g[4])):
        a, b = u + v, roll(u - v)
        re.append(sel(a, b))
        im.append(sel(b, a))
    m1, e = re[0] + re[1], (re[0] - re[1]) * _C5
    t5 = g[0] - m1 * 0.25
    t1, t2 = t5 + e, t5 - e
    t3, t4 = im[0] + im[1] * _R5, im[0] * _R5 - im[1]
    x = [g[0] + m1, t1 + t3, t2 + t4, t2 - t4, t1 - t3]
    return [sel(x[j], x[(j + 3) % 5]) for j in range(5)]


def _build_constants():
    lane = np.arange(128)
    grp = [np.concatenate([c + 10 * np.arange(32) for c in cls]) for cls in _CLASSES]
    d = np.arange(D)[:, None]
    cols = []
    for g, kd in enumerate(grp):
        c, s = np.cos(2 * np.pi * d * kd / D), np.sin(2 * np.pi * d * kd / D)
        if g == 0:
            s[:, 0] = np.cos(np.pi * d[:, 0])
        cols.append(np.concatenate([s, c] if g in (2, 4) else [c, s], axis=1))
    eye = np.eye(D)
    net = np.concatenate(_r10_fwd(
        [eye[:, 128 * j:128 * j + 128] for j in range(NT)],
        lambda a, b: np.where(lane < 64, a, b), lambda a: np.roll(a, 64, axis=1)), axis=1)
    bd = np.linalg.solve(net, np.concatenate(cols, axis=1))
    fd = np.stack([bd[128 * j:128 * j + 128, 128 * j:128 * j + 128] for j in range(NT)])
    assert abs(np.abs(bd).sum() - np.abs(fd).sum()) < 1e-6
    dmat = np.concatenate([fd, fd.transpose(0, 2, 1) / D])
    dmat[NT, ::64] *= 0.5

    cs = [cols[0]] + [np.concatenate(p, axis=1) for j in (1, 3) for p in (
        (cols[j][:, :64], cols[j + 1][:, 64:]), (cols[j][:, 64:], cols[j + 1][:, :64]))]
    net = np.concatenate(_r10_fwd(
        [eye[:, 128 * j:128 * j + 128] for j in range(NT)], None, None), axis=1)
    bd = np.linalg.solve(net, np.concatenate(cs, axis=1))
    f5 = np.stack([bd[128 * i:128 * i + 128, 128 * j:128 * j + 128] for i, j in _PAIRS])
    assert abs(np.abs(bd).sum() - np.abs(f5).sum()) < 1e-6

    leaves = [int(round(th * R1 / (2 * np.pi))) for th, _ in _real_fwd(list(np.eye(R1)))]
    k1 = [min(m, R1 - m) for m in leaves]
    pos = np.arange(128)
    part, n2 = (pos // G) % 2, (pos // (2 * G)) * G + pos % G
    packed = (pos // (2 * G)) * 2 * G + (pos % 2) * G + (pos % (2 * G)) // 2
    fs = []
    for m, kk in zip(leaves, k1):
        ks = (16 * np.arange(R2) if m == 0 else kk + R1 * np.arange(R2))[:, None]
        if m == 0:
            ph = 2 * np.pi * ks * (n2 + R2 * part) / S
            c, s = np.cos(ph), np.sin(ph)
            s[0] = np.cos(np.pi * n2)
        else:
            sg = 1.0 if m == kk else -1.0
            ph = 2 * np.pi * ks * n2 / S
            c = np.where(part == 0, np.cos(ph), -sg * np.sin(ph))
            s = np.where(part == 0, np.sin(ph), sg * np.cos(ph))
        fs.append(np.concatenate([c, s]))
    fs = np.stack(fs)[:, part * R2 + n2]
    smat = np.concatenate([fs[:, :, packed], fs[:, packed].transpose(0, 2, 1) * (2.0 / S)])

    have = np.concatenate([R1 * np.arange(R2), 16 + R1 * (R2 - 1 - np.arange(R2))])
    want = np.concatenate([16 * np.arange(R2), S // 2 + 16 * ((R2 - np.arange(R2)) % R2)])
    p0 = (want[:, None] == have[None, :]).astype(np.float64)

    mats = np.concatenate([f5, smat, p0[None], dmat[NT:], dmat[:NT]]).astype(jnp.bfloat16)
    mats = mats.view(np.uint16).astype(np.uint32)
    return (mats[:, 0::2] | (mats[:, 1::2] << 16)).view(np.int32), k1


_MATS, _K1 = _build_constants()
_F5, _SF, _SI, _P0, _DI, _DF, _NM = 0, 9, 25, 41, 42, 47, 52

F32, BF16, I32 = jnp.float32, jnp.bfloat16, jnp.int32
PITCH = 68
RB = 16
HR = GR // 2
KB = 160
NW = 4
WL = S // NW
LAG = 3
AHEAD = 3
F5 = 7
_MCUT = (0, _SF, _SI, _DI, _DF, _NM)
_HI = np.int32(-65536)
_WIN = ((0, 144), (112, 272), (240, 400), (368, 528), (496, 640))


def _dot(a, b):
    return jnp.dot(a.astype(BF16), b.astype(BF16), preferred_element_type=F32)


def _dot_nt(a, b):
    return lax.dot_general(a.astype(BF16), b.astype(BF16), (((1,), (1,)), ((), ())), preferred_element_type=F32)


def _sel(a, b):
    return jnp.where(lax.broadcasted_iota(I32, a.shape, 1) < 64, a, b)


def _roll(a):
    return pltpu.roll(a, 64, 1)


def _tiles(a):
    return [a[:, 128 * j:128 * j + 128] for j in range(a.shape[1] // 128)]


def _cat(a, axis=0):
    return a[0] if len(a) == 1 else jnp.concatenate(a, axis=axis)


def _split(a):
    return [_cat([a[r:r + G] for r in range(o, a.shape[0], 2 * G)]) for o in (0, G)]


def _merge(a, b):
    return pltpu.pack_elementwise([a, b], packed_dtype=BF16).astype(I32)


def _quads(a, h, w):
    return a[:h, :w], a[:h, w:2 * w], a[h:2 * h, :w], a[h:2 * h, w:2 * w]


def _terms_a(a11, a12, a21, a22):
    return a11 + a22, a22 - a21, a11, a22, a11 - a12, a21 + a11, a12 + a22


def _terms_w(w11, w12, w21, w22):
    return w11 + w22, w11, w12 + w22, w21 + w11, w22, w12 - w11, w21 - w22


_USE = (((0, 1), (3, 1)), ((2, -1), (3, -1)), ((1, 1), (3, -1)), ((0, -1), (2, 1)),
        ((0, -1), (1, -1)), ((3, 1),), ((0, 1),))
_ORD = tuple(int(c) for c in '6403125')
_GORD = tuple(int(c) for c in '780123456')


def _combine(c, p):
    c = list(c)
    for i in reversed(_ORD):
        for k, sg in _USE[i]:
            c[k] = c[k] + p[i] if sg > 0 else c[k] - p[i]
    return c


def _unpack(w):
    return pltpu.bitcast(w & _HI, F32), pltpu.bitcast(w << 16, F32)


def _words(a):
    return pltpu.bitcast(a, I32)


def _phi(t):
    return jnp.where(t > 0, t + 1.0, jnp.exp(t)) + 1e-6


def _ln(x):
    mean = _lane_sum(x[0] + x[1] + x[2] + x[3] + x[4]) * (1.0 / D)
    sq = _lane_sum(x[0] * x[0] + x[1] * x[1] + x[2] * x[2] + x[3] * x[3] + x[4] * x[4])
    r = lax.rsqrt(jnp.maximum(sq * (1.0 / D) - mean * mean, 0.0) + 1e-5)
    return [(a - mean) * r for a in x]


def _lane_sum(a):
    return jnp.sum(a, axis=1, keepdims=True)


def _ln_r5(y0, m1, m2, t3, t4, centred=False):
    mean = _lane_sum(y0) * (1.0 / 128)
    yc = y0 - mean
    sq = (m1 * m1 + m2 * m2) * 4.0 + (t3 * t3 + t4 * t4) * 2.5
    if centred:
        var = _lane_sum(sq + yc * yc) * (0.2 / D)
    else:
        var = jnp.maximum(_lane_sum(sq + y0 * y0) * (0.2 / D) - mean * mean * 0.04, 0.0)
    return yc, lax.rsqrt(var + 1e-5)


def _bf(a):
    return pltpu.bitcast(a, BF16)


def _run(*gens):
    gens = [list(g) for g in gens]
    order = sorted(((i + 0.5) / len(g), k, i) for k, g in enumerate(gens) for i in range(len(g)))
    for _, k, i in order:
        gens[k][i]()


def _zip(a, b):
    n = len(b) // max(len(a), 1)
    return [f for i, p in enumerate(a) for f in [p] + b[i * n:i * n + n]]


def _ds(start, size, align=None):
    if isinstance(start, int):
        return pl.ds(start, size)
    return pl.ds(pl.multiple_of(start, align or size), size)


def _kernel(x_hbm, wr_hbm, wi_hbm, wqkv_hbm, wo_hbm, mats_hbm, o_hbm,
            xio, ybuf, z0, wraw, wtmp, wbuf, wqkv, wo, wqt, zacc, macc, mats, sems, bsem):

    def x_copy(c):
        return pltpu.make_async_copy(x_hbm.at[:, _ds(G * c, G), :], xio.at[c], sems.at[c & 3])

    def o_copy(c, h):
        n1 = pl.ds(h * (R1 // 2), R1 // 2)
        return pltpu.make_async_copy(xio.at[c, n1], o_hbm.at[n1, _ds(G * c, G), :], sems.at[0])

    def w_copy(i, c):
        return pltpu.make_async_copy(
            (wr_hbm, wi_hbm)[i].at[:, _ds(WL * c, WL)], wraw.at[i, c], sems.at[6 + c % 4])

    def m_copy(i):
        lo, hi = _MCUT[i], _MCUT[i + 1]
        return pltpu.make_async_copy(mats_hbm.at[lo:hi], mats.at[lo:hi], sems.at[4 + i % 2])

    def a_copy(k, i):
        rs = pl.ds(128 * i, 128)
        if k == 3:
            return pltpu.make_async_copy(wo_hbm.at[rs], wo.at[rs], sems.at[2])
        return pltpu.make_async_copy(
            wqkv_hbm.at[rs, pl.ds(D * k, D)], wqkv.at[k, rs], sems.at[1 if k == 1 else 2])

    mat = lambda i: _bf(mats[i])
    st = {}

    def fwd_rows(g, r, x):
        st["t", g, r] = _r10_fwd(_tiles(x), _sel if g < F5 else None, _roll, _ln_r5)

    def d5(t, base, j):
        ks = [k for k, p in enumerate(_PAIRS) if p[1] == j]
        return _dot(_cat([t(_PAIRS[k][0]) for k in ks], 1),
                    _cat([mat(base + k) for k in ks]))

    def load_x(g, r, n):
        return _cat([xio[g, i].astype(F32) for i in range(r // G, (r + n) // G)])

    def d_fwd(g):
        def step(j):
            t = lambda i: _cat([st["t", g, r][i] for r in range(0, GR, RB)])
            st["y", g, j] = _dot(t(j).astype(BF16), mat(_DF + j)) if g < F5 else d5(t, _F5, j)
        return [partial(step, j) for j in range(NT)]

    def s_fwd(g, row=None):
        def put(s, j, w):
            if row is None:
                st["z", s, g, j] = w
            else:
                z0[s, _ds(row, G), 128 * j:128 * j + 128] = w

        def step(j):
            y = st["y", g, j]
            v = _real_fwd([y[n * G:n * G + G, :] for n in range(R1)])
            w = [_merge(*p) for _, p in v]
            st["w", g, j] = w
            for s in range(16):
                if j == 0 or g >= F5:
                    put(s, j, w[s])
                elif j % 2 == 0:
                    a, b = st["w", g, j - 1][s], w[s]
                    put(s, j - 1, _sel(a, b))
                    put(s, j, _roll(_sel(b, a)))
        return [partial(step, j) for j in range(NT)]

    def s_bwd(g):
        def step(j):
            r0 = 2 * G * g
            w = _cat(_real_bwd([(st["zi", s, j][r0:r0 + G], st["zi", s, j][r0 + G:r0 + 2 * G])
                                for s in range(16)]))
            st["u", g, j] = w
        return [partial(step, j) for j in range(NT)]

    def d_bwd(g):
        def step(r, j):
            st["v", g, j] = _dot(st["u", g, j][r:r + HR], mat(_DI + j))
            if j == NT - 1:
                _run(bwd_rows(g)[r // RB:(r + HR) // RB])
        return [partial(step, r, j) for r in (0, HR) for j in range(NT)]

    def bwd_rows(g):
        def step(r):
            d = _r10_bwd([st["v", g, j][r % HR:r % HR + RB] for j in range(NT)],
                         _sel, _roll)
            x = st["res", g, r] if ("res", g, r) in st else load_x(g, r, RB)
            x = [a + b for a, b in zip(_tiles(x), d)]
            st["res", g, r] = _cat(x, 1)
            st["xn", g, r] = _cat(_ln(x), 1)
        return [partial(step, r) for r in range(0, GR, RB)]

    def prep_filter(c, t):
        ls = slice(128 * t, 128 * t + 128)

        def merge():
            a, b = _words(wraw[0, c, 0:D // 2, ls]), _words(wraw[1, c, 0:D // 2, ls])
            wtmp[c, t, 0] = (a << 16) | (b & 0xFFFF)
            wtmp[c, t, 1] = (a & _HI) | lax.shift_right_logical(b, 16)

        def step(j):
            cls = lambda k: wtmp[c, t, k % 2, pl.ds(k // 2, 32, stride=5), :]
            if j == 0:
                last = _words(wraw[0, c, D // 2:DF, ls].astype(F32)) | lax.shift_right_logical(
                    _words(wraw[1, c, D // 2:DF, ls].astype(F32)), 16)
                c0, c5 = cls(0), cls(5)
                src = [c0, c5, jnp.where(lax.broadcasted_iota(I32, c0.shape, 0) == 0, last, c0), c5]
            else:
                src = [cls(k) for k in _CLASSES[2 * j - 1] + _CLASSES[2 * j]]
            w = _cat(src).T
            for i in range(16):
                k2, k1 = (WL // R1) * c + 4 * t + i // 4, 8 * (i % 4)
                pos = k2 if k1 < 16 else R2 - 1 - k2
                wbuf[j, pl.ds(k1 * PITCH + pos, 8, stride=PITCH), :] = w[8 * i:8 * i + 8]
        return [merge] + [partial(step, j) for j in range(3)]

    def prep_filter_end():
        for j in range(3):
            w = _cat([wbuf[j, 0:R2, :], wbuf[j, 16 * PITCH:16 * PITCH + R2, :]])
            re = _dot(mat(_P0), pltpu.bitcast(w & _HI, F32).astype(BF16))
            im = _dot(mat(_P0), pltpu.bitcast(w << 16, F32).astype(BF16))
            w = _words(re) | lax.shift_right_logical(_words(im), 16)
            wbuf[j, 0:R2, :] = w[:R2]
            wbuf[j, 16 * PITCH:16 * PITCH + R2, :] = w[R2:]

    def prep_wq(i):
        r0 = (0, 256, 384)[i]
        wqt[i] = _words(wqkv[0, r0:r0 + 256, :]).T
        w = _cat([wqt[i, pl.ds(d, H, stride=DH), :] for d in range(DH)]).T
        st["wq", i] = _bf(w[64:] if i == 2 else w)
        if i == 2:
            w = _cat([st["wq", k] for k in range(3)])
            st["wqs"] = w, _terms_w(*_quads(w.astype(F32), 256, 256))

    def prep_wk(j):
        for k in (0, 2, 1, 3, 4):
            w = wqkv[1, 128 * k:128 * k + 128, 128 * j:128 * j + 128]
            st["wk", j, k] = w.astype(F32).T
        if j == NT - 1:
            w = _cat([_cat([st["wk", i, k][o:o + 64] for k in range(NT)], 1)
                      for o in (0, 64) for i in range(NT)])
            w11, w21, w12, w22 = _quads(w, D // 2, 256)
            st["wkt"], st["wks"] = w, _terms_w(w11, w12, w21, w22)

    def natural(a):
        return _cat([a[o + 64 * i:o + 64 * i + 64] for i in range(NT) for o in (0, D // 2)])

    def masks(s):
        lane = lax.broadcasted_iota(I32, (R2, 128), 1)
        sign = jnp.where((lane & 63) == 0, 0.0, jnp.where(lane < 64, -1.0, 1.0))
        if s:
            return lane, sign, lambda a: a
        row = lax.broadcasted_iota(I32, (R2, 128), 0)
        return lane, sign, lambda a: jnp.where(row == 0, 0.0, a)

    def mid_fwd(s):
        x = []
        for j in range(NT):
            if ("z", s, 0, j) in st:
                a = _cat([st["z", s, g, j] for g in range(NG)])
            else:
                a = z0[s, :, 128 * j:128 * j + 128]
            x.append(_split(_dot(mat(_SF + s), _bf(a))))
        _, sign, m = masks(s)
        st["x", s, 0] = _sel(*x[0]), _sel(*x[0][::-1])
        for j in (1, 3):
            (cc, sc), (cs, ss) = x[j], x[j + 1]
            st["x", s, j] = cc - m(ss), cs + m(sc), m(cc) + ss, m(cs) - sc

    def mid_filter(s):
        k1 = _K1[s]
        p1, p2 = k1 * PITCH, (R1 - k1 if k1 else 16) * PITCH
        lane, sign, m = masks(s)
        a, b = st["x", s, 0]
        re, im = a + m(_roll(a) * sign), m(b) - _roll(b) * sign
        w1, w2 = wbuf[0, p1:p1 + R2, :], wbuf[0, p2:p2 + R2, :]
        (a1, b1), (a2, b2) = _unpack(_sel(w1, w2)), _unpack(
            jnp.where(lane == 0, w2, jnp.where(lane == 64, w1, 0)))
        cr, ci = a1 + a2, b1 - b2
        re, im = cr * re + ci * im, cr * im - ci * re
        an, bn = re - m(_roll(re) * sign), m(im) + _roll(im) * sign
        if not k1:
            corner = (lax.broadcasted_iota(I32, a.shape, 0) + (lane & 63)) == 0
            an, bn = jnp.where(corner, a * a1, an), jnp.where(corner, b * a2, bn)
        out = [_merge(_sel(an, bn), _sel(bn, an))]
        for j in (1, 3):
            r1, n1, r2, n2 = st["x", s, j]
            (a1, b1), (a2, b2) = (_unpack(wbuf[(j + 1) // 2, p:p + R2, :]) for p in (p1, p2))
            r1, n1 = a1 * r1 + b1 * n1, a1 * n1 - b1 * r1
            r2, n2 = a2 * r2 + b2 * n2, a2 * n2 - b2 * r2
            a, b = _merge(r1 + m(r2), m(n1) - n2), _roll(_merge(n1 + m(n2), r2 - m(r1)))
            out += [_sel(a, b), _sel(b, a)]
        st["f", s] = out

    def mid_bwd(s):
        for j in range(NT):
            st["zi", s, j] = _dot(mat(_SI + s), _bf(st["f", s][j]))

    def half(name, h):
        if name != "xn":
            return range(h * HR, h * HR + HR, RB)
        return range(h * RB, GR, 2 * RB)

    def terms(name, g):
        if (name, g) not in st:
            a = _cat([st[name, g, r] for h in (0, 1) for r in half(name, h)])
            st[name, g] = a, _terms_a(*_quads(a, HR, 256))
        return st[name, g]

    def proj(name, g, w, out, fast, then):
        def put(o, y):
            for i, r in enumerate(half(name, o)):
                st[out, g, r] = y[i * RB:i * RB + RB]

        def plain(h):
            put(h, _dot(terms(name, g)[0][h * HR:h * HR + HR], st[w][0]))
            _run([then[r // RB] for r in half(name, h)])

        def side():
            st["e", out] = _dot(terms(name, g)[0], st[w][0][:, 512:])

        def edge():
            c = _dot(terms(name, g)[0][:, 512:], st[w][0][512:, :512])
            c = _combine(_quads(c, HR, 256), [st["c", out, i] for i in range(7)])
            put(0, _cat([c[0], c[1], st["e", out][:HR]], 1))
            put(1, _cat([c[2], c[3], st["e", out][HR:]], 1))
            _run(then)

        def step(i):
            st["c", out, i] = _dot(terms(name, g)[1][i], st[w][1][i])
        if not fast:
            return [partial(plain, h) for h in (0, 1)]
        fs = [partial(step, i) for i in _ORD] + [edge]
        fs.insert(0, side)
        return fs

    def k_mm(g):
        def edge(r):
            e = [_dot_nt(st["wkt"][o:o + KB, 512:], terms("xn", g)[0][:, 512:])
                 for o in (r, D // 2 + r)]
            c = _combine([e[0][:, :HR], e[1][:, :HR], e[0][:, HR:], e[1][:, HR:]],
                         [st["ck", i] for i in range(7)])
            c = [_phi(a) for a in c]
            for o, zs in ((r, c[0] + c[2]), (D // 2 + r, c[1] + c[3])):
                st["zs", o] = st["zs", o] + zs if g else zs
            st["pk", g, r] = ([_cat(c[i::2], 1) for i in (0, 1)],
                              _terms_a(c[0], c[2], c[1], c[3]))

        def step(r, i):
            st["ck", i] = _dot_nt(st["wks"][i][r:r + KB], terms("xn", g)[1][i])
        return [f for r in range(0, D // 2, KB)
                for f in [partial(step, r, i) for i in _ORD] + [partial(edge, r)]]

    def g_mm(g):
        def step(r, i):
            if i < 7:
                a = _dot(st["pk", g, r][1][i], terms("xn", g)[1][(0, 2, 6, 5, 3, 4, 1)[i]])
            else:
                a = _dot(st["pk", g, r][0][i - 7], terms("xn", g)[0][:, 512:])
            st["g", r, i] = st["g", r, i] + a if g else a
        return [partial(step, r, i) for r in range(0, D // 2, KB) for i in _GORD]

    def mix_z():
        zacc[...] = natural(_cat([st["zs", r] for r in range(0, D, KB)]))
        zp = _cat([zacc[pl.ds(d, H, stride=DH), :] for d in range(DH)])
        st["zrow"] = jnp.broadcast_to(jnp.sum(zp.T, axis=0, keepdims=True), (RB, D))

    def mix_kv():
        m1, m2, n3, n4, m5, n6, n7, e0, e1 = (
            _cat([st["g", r, i] for r in range(0, D // 2, KB)]) for i in range(9))
        gm = natural(_cat([_cat([m1 - n4 - m5 - n7, n3 - m5, e0], 1),
                           _cat([n4 - m2, m1 - m2 - n3 - n6, e1], 1)]))
        for j, (r0, r1) in enumerate(_WIN):
            kv = _dot(gm[r0:r1], wqkv[2, :, 128 * j:128 * j + 128])
            hr = ((lax.broadcasted_iota(I32, kv.shape, 0) + r0) * 3277) >> 16
            hc = ((lax.broadcasted_iota(I32, kv.shape, 1) + 128 * j) * 3277) >> 16
            st["kv", j] = jnp.where(hr == hc, kv, 0.0).astype(BF16)

    def mix_m():
        done = 0
        for j, (r0, r1) in enumerate(_WIN):
            m = _dot(st["kv", j], wo[128 * j:128 * j + 128, :])
            for t, a in enumerate(_tiles(m)):
                if done > r0:
                    macc[t, r0:done, :] += a[:done - r0]
                macc[t, done:r1, :] = a[done - r0:]
            done = r1
        w = _cat([_cat([macc[t, pl.ds(d, H, stride=DH), :] for d in range(DH)])
                  for t in range(NT)], 1)
        st["m"] = w, _terms_w(*_quads(w, 256, 256))

    def q_mm(g):
        return proj("xn", g, "wqs", "q", True, q_act(g))

    def q_act(g):
        def step(r):
            zt = _tiles(st["zrow"])
            p = _tiles(_phi(st["q", g, r]))
            den = p[0] * zt[0] + p[1] * zt[1] + p[2] * zt[2] + p[3] * zt[3] + p[4] * zt[4]
            den = den + _roll(den)
            den = den + pltpu.roll(den, 32, 1)
            inv = 1.0 / (den + 1e-6)
            st["p", g, r] = _cat([a * inv for a in p], 1)
        return [partial(step, r) for r in range(0, GR, RB)]

    def o_mm(g, last):
        return proj("p", g, "m", "o", last and g < 7, o_rows(g, last))

    def o_rows(g, last):
        def step(r):
            x = st["res", g, r] + st["o", g, r]
            if last:
                for i in range(0, RB, G):
                    xio[g, (r + i) // G] = x[i:i + G].astype(BF16)
                if (r + RB) % HR == 0:
                    o_copy(g, r // HR).start()
            else:
                st["res", g, r] = x
                fwd_rows(g, r, x)
        return [partial(step, r) for r in range(0, GR, RB)]

    def fence():
        pl.semaphore_signal(bsem)
        pl.semaphore_wait(bsem)

    def at(f, g, *a):
        return f(g, *a) if 0 <= g < NG else []

    def rows(c):
        t = _r10_fwd(_tiles(load_x(c, 0, GR)), None, None, partial(_ln_r5, centred=True))
        for j in range(NT):
            ybuf[j] = t[j]

    def cols(c):
        for j in range(NT):
            st["y", NG, j] = d5(lambda i: ybuf[i], _F5, j)
        return s_fwd(NG, G * c)

    def filt(c):
        w_copy(0, c).wait()
        w_copy(1, c).wait()
        return sum([prep_filter(c, t) for t in range(WL // 128)], [])

    def w_start(c):
        w_copy(0, c).start()
        w_copy(1, c).start()

    def first(c, _):
        x_copy(c).wait()
        pl.when(c + AHEAD < NG)(lambda: x_copy(c + AHEAD).start())
        pl.when(c == NG - 2)(lambda: m_copy(1).start())
        for i in range(NW):
            pl.when(c == NG - NW + i)(partial(w_start, i))
        _run([partial(rows, c)], cols(c - 1))

    x_copy(0).start()
    m_copy(0).start()
    x_copy(1).start()
    x_copy(0).wait()
    for c in range(2, AHEAD + 1):
        x_copy(c).start()
    rows(0)
    m_copy(0).wait()
    lax.fori_loop(1, NG, first, None)

    order = list(range(1, 16)) + [0]
    for c in range(NW):
        if c == 1:
            m_copy(1).wait()
        pf = filt(c)
        if c == 0:
            m_copy(2).start()
        if c == NW - 1:
            m_copy(3).start()
            for j in range(NT):
                a_copy(1, j).start()
        _run(pf, [partial(mid_fwd, s) for s in order[6 * c - 6:6 * c]] if c else cols(NG - 1))
    m_copy(2).wait()

    nop = lambda: None
    for layer in range(2):
        for g in range(NG):
            st.pop(("xn", g), None)
            st.pop(("p", g), None)
        for i in range(16 + LAG):
            if layer == 0 and i == 2:
                prep_filter_end()
            if layer == 0 and i == 15 + LAG:
                m_copy(3).wait()
                for j in range(NT):
                    a_copy(1, j).wait()
                m_copy(4).start()
            if layer and i < 16:
                mid_fwd(order[i])
            if i >= LAG:
                mid_bwd(order[i - LAG])
            if i < 16:
                mid_filter(order[i])
        fence()
        for g in range(NG + 2):
            if layer == 0:
                if g == 0:
                    for j in range(NT):
                        prep_wk(j)
                if 1 <= g <= NT:
                    wqkv[0, 128 * g - 128:128 * g - 112, :128] = (
                        st["xn", g - 1, 0][:, :128].astype(BF16))
                    for k in (0, 2, 3):
                        a_copy(k, g - 1).start()
                if g == NG:
                    m_copy(4).wait()
                    for k in (0, 2, 3):
                        for j in range(NT):
                            a_copy(k, j).wait()
                    prep_wq(0)
                if g == NG + 1:
                    prep_wq(1)
                    prep_wq(2)
            _run(at(s_bwd, g))
            _run(at(d_bwd, g) + [nop] * 5, [nop] * 0 + at(g_mm, g - 2) + [nop] * 0,
                 [nop] * 0 + at(k_mm, g - 1) + [nop] * 0)
        if layer:
            fence()
        mix_z()
        _run(q_mm(0))
        mix_kv()
        mix_m()
        _run(q_mm(1))
        for g in range(NG + 1):
            dm = [] if layer else _zip(at(d_fwd, g - 1), at(s_fwd, g - 1))
            _run((at(q_mm, g + 1) if g else []) + at(o_mm, g, layer == 1), [nop] * 6 + dm + [nop] * 2)
    for c in range(NG):
        o_copy(c, 0).wait()
        o_copy(c, 1).wait()


@jax.jit
def pallas_interleave_layers__spectral_gfnet__linear_attn_block__prompt_kernel(
    A_x, A_w_r, A_w_i, B_x, B_wqkv, B_wo
):
    del B_x
    vm = pltpu.VMEM
    out = pl.pallas_call(
        _kernel,
        in_specs=[pl.BlockSpec(memory_space=pl.ANY)] * 6,
        out_specs=pl.BlockSpec(memory_space=pl.ANY),
        out_shape=jax.ShapeDtypeStruct((R1, R2, D), BF16),
        scratch_shapes=[
            vm((NG, R1, G, D), BF16),
            vm((NT, GR, 128), F32),
            vm((16, R2, D), I32),
            vm((2, S // WL, DF, WL), BF16),
            vm((NW, WL // 128, 2, D // 4, 128), I32),
            vm((3, R1 * PITCH, 128), I32),
            vm((3, D, D), BF16),
            vm((D, D), BF16),
            vm((3, D, 128), I32),
            vm((D, 128), F32),
            vm((NT, D, 128), F32),
            vm(_MATS.shape, I32),
            pltpu.SemaphoreType.DMA((10,)),
            pltpu.SemaphoreType.REGULAR,
        ],
        compiler_params=pltpu.CompilerParams(vmem_limit_bytes=100 * 1024 * 1024),
    )(A_x.reshape(R1, R2, D), A_w_r.T, A_w_i.T, B_wqkv, B_wo, _MATS)
    return out.reshape(1, S, D)
```

```python
from functools import partial

import numpy as np
import jax
import jax.numpy as jnp
from jax import lax
import jax.experimental.pallas as pl
import jax.experimental.pallas.tpu as pltpu

S, D, H, DH = 2048, 640, 32, 20
DF = D // 2 + 1
R1, R2 = 32, 64
G = 8
NG = R2 // G
GR = R1 * G
NT = D // 128

_C5 = float(np.sqrt(5.0) / 4.0)
_R5 = float(np.sin(4 * np.pi / 5) / np.sin(2 * np.pi / 5))
_PAIRS = ((0, 0), (1, 1), (2, 1), (1, 2), (2, 2), (3, 3), (4, 3), (3, 4), (4, 4))
_CLASSES = ((0, 5), (4, 6), (1, 9), (2, 8), (3, 7))


def _cmul(re, im, ang):
    c, s = float(np.cos(ang)), float(np.sin(ang))
    if abs(abs(c) - abs(s)) < 1e-12:
        if c * s > 0:
            return (re - im) * c, (re + im) * c
        return (re + im) * c, (im - re) * c
    return re * c - im * s, re * s + im * c


def _cadd(p, q):
    return p[0] + q[0], p[1] + q[1]


def _csub(p, q):
    return p[0] - q[0], p[1] - q[1]


def _cplx_fwd(u, th):
    n = len(u)
    if n == 1:
        return [(th, u[0])]
    if n == 4:
        v1, v2, v3 = (_cmul(*u[k], k * th / 4) for k in (1, 2, 3))
        a, b, c, d = _cadd(u[0], v2), _csub(u[0], v2), _cadd(v1, v3), _csub(v1, v3)
        out = _cadd(a, c), _csub(a, c), (b[0] - d[1], b[1] + d[0]), (b[0] + d[1], b[1] - d[0])
        return [(th / 4 + k * np.pi / 2, o) for k, o in zip((0, 2, 1, 3), out)]
    h = n // 2
    v = [_cmul(re, im, th / 2) for re, im in u[h:]]
    a = [_cadd(p, q) for p, q in zip(u[:h], v)]
    b = [_csub(p, q) for p, q in zip(u[:h], v)]
    return _cplx_fwd(a, th / 2) + _cplx_fwd(b, th / 2 + np.pi)


def _cplx_bwd(g, th):
    n = len(g)
    if n == 1:
        return list(g)
    if n == 4:
        a, c, b = _cadd(g[0], g[1]), _csub(g[0], g[1]), _cadd(g[2], g[3])
        d = (g[2][1] - g[3][1], g[3][0] - g[2][0])
        v = _cadd(c, d), _csub(a, b), _csub(c, d)
        return [_cadd(a, b)] + [_cmul(*v[k - 1], -k * th / 4) for k in (1, 2, 3)]
    h = n // 2
    a, b = _cplx_bwd(g[:h], th / 2), _cplx_bwd(g[h:], th / 2 + np.pi)
    return [_cadd(p, q) for p, q in zip(a, b)] + [
        _cmul(*_csub(p, q), -th / 2) for p, q in zip(a, b)]


def _real_fwd(x):
    n = len(x)
    if n == 2:
        return [(0.0, (x[0], x[1]))]
    h, q = n // 2, n // 4
    a = [x[j] + x[j + h] for j in range(h)]
    b = [x[j] - x[j + h] for j in range(h)]
    return _real_fwd(a) + _cplx_fwd([(b[j], b[j + q]) for j in range(q)], np.pi / 2)


def _real_bwd(g):
    if len(g) == 1:
        return list(g[0])
    h = len(g) // 2
    a = _real_bwd(g[:h])
    u = _cplx_bwd(g[h:], np.pi / 2)
    b = [p[0] for p in u] + [p[1] for p in u]
    return [p + q for p, q in zip(a, b)] + [p - q for p, q in zip(a, b)]


def _r10_fwd(x, sel, roll, norm=None):
    if sel is not None:
        x = [sel(x[j], x[(j + 2) % 5]) for j in range(5)]
    t1, t2, t3, t4 = x[1] + x[4], x[2] + x[3], x[1] - x[4], x[2] - x[3]
    t5 = t1 + t2
    y0, m1, m2 = x[0] + t5, x[0] - t5 * 0.25, (t1 - t2) * _C5
    out = []
    for re, im in ((m1 + m2, t3 + t4 * _R5), (m1 - m2, t3 * _R5 - t4)):
        if sel is None:
            out += [re, im]
        else:
            a, b = sel(re, im), roll(sel(im, re))
            out += [a + b, a - b]
    if norm is None:
        return [y0] + out
    y0, scale = norm(y0, m1, m2, t3, t4)
    return [a * scale for a in [y0] + out]


def _r10_bwd(g, sel, roll):
    re, im = [], []
    for u, v in ((g[1], g[2]), (g[3], g[4])):
        a, b = u + v, roll(u - v)
        re.append(sel(a, b))
        im.append(sel(b, a))
    m1, e = re[0] + re[1], (re[0] - re[1]) * _C5
    t5 = g[0] - m1 * 0.25
    t1, t2 = t5 + e, t5 - e
    t3, t4 = im[0] + im[1] * _R5, im[0] * _R5 - im[1]
    x = [g[0] + m1, t1 + t3, t2 + t4, t2 - t4, t1 - t3]
    return [sel(x[j], x[(j + 3) % 5]) for j in range(5)]


def _build_constants():
    lane = np.arange(128)
    grp = [np.concatenate([c + 10 * np.arange(32) for c in cls]) for cls in _CLASSES]
    d = np.arange(D)[:, None]
    cols = []
    for g, kd in enumerate(grp):
        c, s = np.cos(2 * np.pi * d * kd / D), np.sin(2 * np.pi * d * kd / D)
        if g == 0:
            s[:, 0] = np.cos(np.pi * d[:, 0])
        cols.append(np.concatenate([s, c] if g in (2, 4) else [c, s], axis=1))
    eye = np.eye(D)
    net = np.concatenate(_r10_fwd(
        [eye[:, 128 * j:128 * j + 128] for j in range(NT)],
        lambda a, b: np.where(lane < 64, a, b), lambda a: np.roll(a, 64, axis=1)), axis=1)
    bd = np.linalg.solve(net, np.concatenate(cols, axis=1))
    fd = np.stack([bd[128 * j:128 * j + 128, 128 * j:128 * j + 128] for j in range(NT)])
    assert abs(np.abs(bd).sum() - np.abs(fd).sum()) < 1e-6
    dmat = np.concatenate([fd, fd.transpose(0, 2, 1) / D])
    dmat[NT, ::64] *= 0.5

    cs = [cols[0]] + [np.concatenate(p, axis=1) for j in (1, 3) for p in (
        (cols[j][:, :64], cols[j + 1][:, 64:]), (cols[j][:, 64:], cols[j + 1][:, :64]))]
    net = np.concatenate(_r10_fwd(
        [eye[:, 128 * j:128 * j + 128] for j in range(NT)], None, None), axis=1)
    bd = np.linalg.solve(net, np.concatenate(cs, axis=1))
    f5 = np.stack([bd[128 * i:128 * i + 128, 128 * j:128 * j + 128] for i, j in _PAIRS])
    assert abs(np.abs(bd).sum() - np.abs(f5).sum()) < 1e-6

    leaves = [int(round(th * R1 / (2 * np.pi))) for th, _ in _real_fwd(list(np.eye(R1)))]
    k1 = [min(m, R1 - m) for m in leaves]
    pos = np.arange(128)
    part, n2 = (pos // G) % 2, (pos // (2 * G)) * G + pos % G
    packed = (pos // (2 * G)) * 2 * G + (pos % 2) * G + (pos % (2 * G)) // 2
    fs = []
    for m, kk in zip(leaves, k1):
        ks = (16 * np.arange(R2) if m == 0 else kk + R1 * np.arange(R2))[:, None]
        if m == 0:
            ph = 2 * np.pi * ks * (n2 + R2 * part) / S
            c, s = np.cos(ph), np.sin(ph)
            s[0] = np.cos(np.pi * n2)
        else:
            sg = 1.0 if m == kk else -1.0
            ph = 2 * np.pi * ks * n2 / S
            c = np.where(part == 0, np.cos(ph), -sg * np.sin(ph))
            s = np.where(part == 0, np.sin(ph), sg * np.cos(ph))
        fs.append(np.concatenate([c, s]))
    fs = np.stack(fs)[:, part * R2 + n2]
    smat = np.concatenate([fs[:, :, packed], fs[:, packed].transpose(0, 2, 1) * (2.0 / S)])

    have = np.concatenate([R1 * np.arange(R2), 16 + R1 * (R2 - 1 - np.arange(R2))])
    want = np.concatenate([16 * np.arange(R2), S // 2 + 16 * ((R2 - np.arange(R2)) % R2)])
    p0 = (want[:, None] == have[None, :]).astype(np.float64)

    mats = np.concatenate([f5, smat, p0[None], dmat[NT:], dmat[:NT]]).astype(jnp.bfloat16)
    mats = mats.view(np.uint16).astype(np.uint32)
    return (mats[:, 0::2] | (mats[:, 1::2] << 16)).view(np.int32), k1


_MATS, _K1 = _build_constants()
_F5, _SF, _SI, _P0, _DI, _DF, _NM = 0, 9, 25, 41, 42, 47, 52

F32, BF16, I32 = jnp.float32, jnp.bfloat16, jnp.int32
PITCH = 68
RB = 16
HR = GR // 2
KB = 160
NW = 4
WL = S // NW
LAG = 3
AHEAD = 3
F5 = 7
_MCUT = (0, _SF, _SI, _DI, _DF, _NM)
_HI = np.int32(-65536)
_WIN = ((0, 144), (112, 272), (240, 400), (368, 528), (496, 640))


def _dot(a, b):
    return jnp.dot(a.astype(BF16), b.astype(BF16), preferred_element_type=F32)


def _dot_nt(a, b):
    return lax.dot_general(a.astype(BF16), b.astype(BF16), (((1,), (1,)), ((), ())), preferred_element_type=F32)


def _sel(a, b):
    return jnp.where(lax.broadcasted_iota(I32, a.shape, 1) < 64, a, b)


def _roll(a):
    return pltpu.roll(a, 64, 1)


def _tiles(a):
    return [a[:, 128 * j:128 * j + 128] for j in range(a.shape[1] // 128)]


def _cat(a, axis=0):
    return a[0] if len(a) == 1 else jnp.concatenate(a, axis=axis)


def _split(a):
    return [_cat([a[r:r + G] for r in range(o, a.shape[0], 2 * G)]) for o in (0, G)]


def _merge(a, b):
    return pltpu.pack_elementwise([a, b], packed_dtype=BF16).astype(I32)


def _quads(a, h, w):
    return a[:h, :w], a[:h, w:2 * w], a[h:2 * h, :w], a[h:2 * h, w:2 * w]


def _terms_a(a11, a12, a21, a22):
    return a11 + a22, a22 - a21, a11, a22, a11 - a12, a21 + a11, a12 + a22


def _terms_w(w11, w12, w21, w22):
    return w11 + w22, w11, w12 + w22, w21 + w11, w22, w12 - w11, w21 - w22


_USE = (((0, 1), (3, 1)), ((2, -1), (3, -1)), ((1, 1), (3, -1)), ((0, -1), (2, 1)),
        ((0, -1), (1, -1)), ((3, 1),), ((0, 1),))
_ORD = (6, 4, 0, 3, 1, 2, 5)
_GORD = (0, 1, 6, 2, 3, 4, 5, 7, 8)


def _combine(c, p):
    c = list(c)
    for i in reversed(_ORD):
        for k, sg in _USE[i]:
            c[k] = c[k] + p[i] if sg > 0 else c[k] - p[i]
    return c


def _unpack(w):
    return pltpu.bitcast(w & _HI, F32), pltpu.bitcast(w << 16, F32)


def _words(a):
    return pltpu.bitcast(a, I32)


def _phi(t):
    return jnp.where(t > 0, t + 1.0, jnp.exp(t)) + 1e-6


def _ln(x):
    mean = _lane_sum(x[0] + x[1] + x[2] + x[3] + x[4]) * (1.0 / D)
    sq = _lane_sum(x[0] * x[0] + x[1] * x[1] + x[2] * x[2] + x[3] * x[3] + x[4] * x[4])
    r = lax.rsqrt(jnp.maximum(sq * (1.0 / D) - mean * mean, 0.0) + 1e-5)
    return [(a - mean) * r for a in x]


def _lane_sum(a):
    return jnp.sum(a, axis=1, keepdims=True)


def _ln_r5(y0, m1, m2, t3, t4, centred=False):
    mean = _lane_sum(y0) * (1.0 / 128)
    yc = y0 - mean
    sq = (m1 * m1 + m2 * m2) * 4.0 + (t3 * t3 + t4 * t4) * 2.5
    if centred:
        var = _lane_sum(sq + yc * yc) * (0.2 / D)
    else:
        var = jnp.maximum(_lane_sum(sq + y0 * y0) * (0.2 / D) - mean * mean * 0.04, 0.0)
    return yc, lax.rsqrt(var + 1e-5)


def _bf(a):
    return pltpu.bitcast(a, BF16)


def _run(*gens):
    gens = [list(g) for g in gens]
    order = sorted(((i + 0.5) / len(g), k, i) for k, g in enumerate(gens) for i in range(len(g)))
    for _, k, i in order:
        gens[k][i]()


def _zip(a, b):
    n = len(b) // max(len(a), 1)
    return [f for i, p in enumerate(a) for f in [p] + b[i * n:i * n + n]]


def _ds(start, size, align=None):
    if isinstance(start, int):
        return pl.ds(start, size)
    return pl.ds(pl.multiple_of(start, align or size), size)


def _kernel(x_hbm, wr_hbm, wi_hbm, wqkv_hbm, wo_hbm, mats_hbm, o_hbm,
            xio, ybuf, z0, wraw, wtmp, wbuf, wqkv, wo, wqt, zacc, macc, mats, sems, bsem):

    def x_copy(c):
        return pltpu.make_async_copy(x_hbm.at[:, _ds(G * c, G), :], xio.at[c], sems.at[c & 3])

    def o_copy(c, h):
        n1 = pl.ds(h * (R1 // 2), R1 // 2)
        return pltpu.make_async_copy(xio.at[c, n1], o_hbm.at[n1, _ds(G * c, G), :], sems.at[0])

    def w_copy(i, c):
        return pltpu.make_async_copy(
            (wr_hbm, wi_hbm)[i].at[:, _ds(WL * c, WL)], wraw.at[i, c], sems.at[6 + c % 4])

    def m_copy(i):
        lo, hi = _MCUT[i], _MCUT[i + 1]
        return pltpu.make_async_copy(mats_hbm.at[lo:hi], mats.at[lo:hi], sems.at[4 + i % 2])

    def a_copy(k, i):
        rs = pl.ds(128 * i, 128)
        if k == 3:
            return pltpu.make_async_copy(wo_hbm.at[rs], wo.at[rs], sems.at[2])
        return pltpu.make_async_copy(
            wqkv_hbm.at[rs, pl.ds(D * k, D)], wqkv.at[k, rs], sems.at[1 if k == 1 else 2])

    mat = lambda i: _bf(mats[i])
    st = {}

    def fwd_rows(g, r, x):
        st["t", g, r] = _r10_fwd(_tiles(x), _sel if g < F5 else None, _roll, _ln_r5)

    def d5(t, base, j):
        ks = [k for k, p in enumerate(_PAIRS) if p[1] == j]
        return _dot(_cat([t(_PAIRS[k][0]) for k in ks], 1),
                    _cat([mat(base + k) for k in ks]))

    def load_x(g, r, n):
        return _cat([xio[g, i].astype(F32) for i in range(r // G, (r + n) // G)])

    def d_fwd(g):
        def step(j):
            t = lambda i: _cat([st["t", g, r][i] for r in range(0, GR, RB)])
            st["y", g, j] = _dot(t(j).astype(BF16), mat(_DF + j)) if g < F5 else d5(t, _F5, j)
        return [partial(step, j) for j in range(NT)]

    def s_fwd(g, row=None):
        def put(s, j, w):
            if row is None:
                st["z", s, g, j] = w
            else:
                z0[s, _ds(row, G), 128 * j:128 * j + 128] = w

        def step(j):
            y = st["y", g, j]
            v = _real_fwd([y[n * G:n * G + G, :] for n in range(R1)])
            w = [_merge(*p) for _, p in v]
            st["w", g, j] = w
            for s in range(16):
                if j == 0 or g >= F5:
                    put(s, j, w[s])
                elif j % 2 == 0:
                    a, b = st["w", g, j - 1][s], w[s]
                    put(s, j - 1, _sel(a, b))
                    put(s, j, _roll(_sel(b, a)))
        return [partial(step, j) for j in range(NT)]

    def s_bwd(g):
        def step(j):
            r0 = 2 * G * g
            w = _cat(_real_bwd([(st["zi", s, j][r0:r0 + G], st["zi", s, j][r0 + G:r0 + 2 * G])
                                for s in range(16)]))
            st["u", g, j] = w
        return [partial(step, j) for j in range(NT)]

    def d_bwd(g):
        def step(r, j):
            st["v", g, j] = _dot(st["u", g, j][r:r + HR], mat(_DI + j))
            if j == NT - 1:
                _run(bwd_rows(g)[r // RB:(r + HR) // RB])
        return [partial(step, r, j) for r in (0, HR) for j in range(NT)]

    def bwd_rows(g):
        def step(r):
            d = _r10_bwd([st["v", g, j][r % HR:r % HR + RB] for j in range(NT)],
                         _sel, _roll)
            x = st["res", g, r] if ("res", g, r) in st else load_x(g, r, RB)
            x = [a + b for a, b in zip(_tiles(x), d)]
            st["res", g, r] = _cat(x, 1)
            st["xn", g, r] = _cat(_ln(x), 1)
        return [partial(step, r) for r in range(0, GR, RB)]

    def prep_filter(c, t):
        ls = slice(128 * t, 128 * t + 128)

        def merge():
            a, b = _words(wraw[0, c, 0:D // 2, ls]), _words(wraw[1, c, 0:D // 2, ls])
            wtmp[c, t, 0, :D // 4] = (a << 16) | (b & 0xFFFF)
            wtmp[c, t, 1, :D // 4] = (a & _HI) | lax.shift_right_logical(b, 16)

        def step(j):
            cls = lambda k: wtmp[c, t, k % 2, pl.ds(k // 2, 32, stride=5), :]
            if j == 0:
                last = _words(wraw[0, c, D // 2:DF, ls].astype(F32)) | lax.shift_right_logical(
                    _words(wraw[1, c, D // 2:DF, ls].astype(F32)), 16)
                c0, c5 = cls(0), cls(5)
                src = [c0, c5, jnp.where(lax.broadcasted_iota(I32, c0.shape, 0) == 0, last, c0), c5]
            else:
                src = [cls(k) for k in _CLASSES[2 * j - 1] + _CLASSES[2 * j]]
            w = _cat(src).T
            for i in range(16):
                k2, k1 = (WL // R1) * c + 4 * t + i // 4, 8 * (i % 4)
                pos = k2 if k1 < 16 else R2 - 1 - k2
                wbuf[j, pl.ds(k1 * PITCH + pos, 8, stride=PITCH), :] = w[8 * i:8 * i + 8]
        return [merge] + [partial(step, j) for j in range(3)]

    def prep_filter_end():
        for j in range(3):
            w = _cat([wbuf[j, 0:R2, :], wbuf[j, 16 * PITCH:16 * PITCH + R2, :]])
            re = _dot(mat(_P0), pltpu.bitcast(w & _HI, F32).astype(BF16))
            im = _dot(mat(_P0), pltpu.bitcast(w << 16, F32).astype(BF16))
            w = _words(re) | lax.shift_right_logical(_words(im), 16)
            wbuf[j, 0:R2, :] = w[:R2]
            wbuf[j, 16 * PITCH:16 * PITCH + R2, :] = w[R2:]

    def prep_wq(i):
        r0 = (0, 256, 384)[i]
        wqt[i, :D] = _words(wqkv[0, r0:r0 + 256, :]).T
        w = _cat([wqt[i, pl.ds(d, H, stride=DH), :] for d in range(DH)]).T
        st["wq", i] = _bf(w[64:] if i == 2 else w)
        if i == 2:
            w = _cat([st["wq", k] for k in range(3)])
            st["wqs"] = w, _terms_w(*_quads(w.astype(F32), 256, 256))

    def prep_wk(j):
        for k in (0, 2, 1, 3, 4):
            w = wqkv[1, 128 * k:128 * k + 128, 128 * j:128 * j + 128]
            st["wk", j, k] = w.astype(F32).T
        if j == NT - 1:
            w = _cat([_cat([st["wk", i, k][o:o + 64] for k in range(NT)], 1)
                      for o in (0, 64) for i in range(NT)])
            w11, w21, w12, w22 = _quads(w, D // 2, 256)
            st["wkt"], st["wks"] = w, _terms_w(w11, w12, w21, w22)

    def natural(a):
        return _cat([a[o + 64 * i:o + 64 * i + 64] for i in range(NT) for o in (0, D // 2)])

    def masks(s):
        lane = lax.broadcasted_iota(I32, (R2, 128), 1)
        sign = jnp.where((lane & 63) == 0, 0.0, jnp.where(lane < 64, -1.0, 1.0))
        if s:
            return lane, sign, lambda a: a
        row = lax.broadcasted_iota(I32, (R2, 128), 0)
        return lane, sign, lambda a: jnp.where(row == 0, 0.0, a)

    def mid_fwd(s):
        x = []
        for j in range(NT):
            if ("z", s, 0, j) in st:
                a = _cat([st["z", s, g, j] for g in range(NG)])
            else:
                a = z0[s, :, 128 * j:128 * j + 128]
            x.append(_split(_dot(mat(_SF + s), _bf(a))))
        _, sign, m = masks(s)
        st["x", s, 0] = _sel(*x[0]), _sel(*x[0][::-1])
        for j in (1, 3):
            (cc, sc), (cs, ss) = x[j], x[j + 1]
            st["x", s, j] = cc - m(ss), cs + m(sc), m(cc) + ss, m(cs) - sc

    def mid_filter(s):
        k1 = _K1[s]
        p1, p2 = k1 * PITCH, (R1 - k1 if k1 else 16) * PITCH
        lane, sign, m = masks(s)
        a, b = st["x", s, 0]
        re, im = a + m(_roll(a) * sign), m(b) - _roll(b) * sign
        w1, w2 = wbuf[0, p1:p1 + R2, :], wbuf[0, p2:p2 + R2, :]
        (a1, b1), (a2, b2) = _unpack(_sel(w1, w2)), _unpack(
            jnp.where(lane == 0, w2, jnp.where(lane == 64, w1, 0)))
        cr, ci = a1 + a2, b1 - b2
        re, im = cr * re + ci * im, cr * im - ci * re
        an, bn = re - m(_roll(re) * sign), m(im) + _roll(im) * sign
        if not k1:
            corner = (lax.broadcasted_iota(I32, a.shape, 0) + (lane & 63)) == 0
            an, bn = jnp.where(corner, a * a1, an), jnp.where(corner, b * a2, bn)
        out = [_merge(_sel(an, bn), _sel(bn, an))]
        for j in (1, 3):
            r1, n1, r2, n2 = st["x", s, j]
            (a1, b1), (a2, b2) = (_unpack(wbuf[(j + 1) // 2, p:p + R2, :]) for p in (p1, p2))
            r1, n1 = a1 * r1 + b1 * n1, a1 * n1 - b1 * r1
            r2, n2 = a2 * r2 + b2 * n2, a2 * n2 - b2 * r2
            a, b = _merge(r1 + m(r2), m(n1) - n2), _roll(_merge(n1 + m(n2), r2 - m(r1)))
            out += [_sel(a, b), _sel(b, a)]
        st["f", s] = out

    def mid_bwd(s):
        for j in range(NT):
            st["zi", s, j] = _dot(mat(_SI + s), _bf(st["f", s][j]))

    def half(name, h):
        if name != "xn":
            return range(h * HR, h * HR + HR, RB)
        return range(h * RB, GR, 2 * RB)

    def terms(name, g):
        if (name, g) not in st:
            a = _cat([st[name, g, r] for h in (0, 1) for r in half(name, h)])
            st[name, g] = a, _terms_a(*_quads(a, HR, 256))
        return st[name, g]

    def proj(name, g, w, out, fast, then):
        def put(o, y):
            for i, r in enumerate(half(name, o)):
                st[out, g, r] = y[i * RB:i * RB + RB]

        def plain(h):
            put(h, _dot(terms(name, g)[0][h * HR:h * HR + HR], st[w][0]))
            _run([then[r // RB] for r in half(name, h)])

        def side():
            st["e", out] = _dot(terms(name, g)[0], st[w][0][:, 512:])

        def edge():
            c = _dot(terms(name, g)[0][:, 512:], st[w][0][512:, :512])
            c = _combine(_quads(c, HR, 256), [st["c", out, i] for i in range(7)])
            put(0, _cat([c[0], c[1], st["e", out][:HR]], 1))
            put(1, _cat([c[2], c[3], st["e", out][HR:]], 1))
            _run(then)

        def step(i):
            st["c", out, i] = _dot(terms(name, g)[1][i], st[w][1][i])
        if not fast:
            return [partial(plain, h) for h in (0, 1)]
        return [side] + [partial(step, i) for i in _ORD] + [edge]

    def k_mm(g):
        def edge(r):
            e = [_dot_nt(st["wkt"][o:o + KB, 512:], terms("xn", g)[0][:, 512:])
                 for o in (r, D // 2 + r)]
            c = _combine([e[0][:, :HR], e[1][:, :HR], e[0][:, HR:], e[1][:, HR:]],
                         [st["ck", i] for i in range(7)])
            c = [_phi(a) for a in c]
            for o, zs in ((r, c[0] + c[2]), (D // 2 + r, c[1] + c[3])):
                st["zs", o] = st["zs", o] + zs if g else zs
            st["pk", g, r] = ([_cat(c[i::2], 1) for i in (0, 1)],
                              _terms_a(c[0], c[2], c[1], c[3]))

        def step(r, i):
            st["ck", i] = _dot_nt(st["wks"][i][r:r + KB], terms("xn", g)[1][i])
        return [f for r in range(0, D // 2, KB)
                for f in [partial(step, r, i) for i in _ORD] + [partial(edge, r)]]

    def g_mm(g):
        def step(r, i):
            if i < 7:
                a = _dot(st["pk", g, r][1][i], terms("xn", g)[1][(0, 2, 6, 5, 3, 4, 1)[i]])
            else:
                a = _dot(st["pk", g, r][0][i - 7], terms("xn", g)[0][:, 512:])
            st["g", r, i] = st["g", r, i] + a if g else a
        return [partial(step, r, i) for r in range(0, D // 2, KB) for i in _GORD]

    def mix_z():
        zacc[:D] = natural(_cat([st["zs", r] for r in range(0, D, KB)]))
        zp = _cat([zacc[pl.ds(d, H, stride=DH), :] for d in range(DH)])
        st["zrow"] = jnp.broadcast_to(jnp.sum(zp.T, axis=0, keepdims=True), (RB, D))

    def mix_kv():
        m1, m2, n3, n4, m5, n6, n7, e0, e1 = (
            _cat([st["g", r, i] for r in range(0, D // 2, KB)]) for i in range(9))
        gm = natural(_cat([_cat([m1 - n4 - m5 - n7, n3 - m5, e0], 1),
                           _cat([n4 - m2, m1 - m2 - n3 - n6, e1], 1)]))
        for j, (r0, r1) in enumerate(_WIN):
            kv = _dot(gm[r0:r1], wqkv[2, :, 128 * j:128 * j + 128])
            hr = ((lax.broadcasted_iota(I32, kv.shape, 0) + r0) * 3277) >> 16
            hc = ((lax.broadcasted_iota(I32, kv.shape, 1) + 128 * j) * 3277) >> 16
            st["kv", j] = jnp.where(hr == hc, kv, 0.0).astype(BF16)

    def mix_m():
        done = 0
        for j, (r0, r1) in enumerate(_WIN):
            m = _dot(st["kv", j], wo[128 * j:128 * j + 128, :])
            for t, a in enumerate(_tiles(m)):
                if done > r0:
                    macc[t, r0:done, :] += a[:done - r0]
                macc[t, done:r1, :] = a[done - r0:]
            done = r1
        w = _cat([_cat([macc[t, pl.ds(d, H, stride=DH), :] for d in range(DH)])
                  for t in range(NT)], 1)
        st["m"] = w, _terms_w(*_quads(w, 256, 256))

    def q_mm(g):
        return proj("xn", g, "wqs", "q", True, q_act(g))

    def q_act(g):
        def step(r):
            zt = _tiles(st["zrow"])
            p = _tiles(_phi(st["q", g, r]))
            den = p[0] * zt[0] + p[1] * zt[1] + p[2] * zt[2] + p[3] * zt[3] + p[4] * zt[4]
            den = den + _roll(den)
            den = den + pltpu.roll(den, 32, 1)
            den = den + 1e-6
            inv = pl.reciprocal(den, approx=True)
            inv = inv * (2.0 - den * inv)
            st["p", g, r] = _cat([a * inv for a in p], 1)
        return [partial(step, r) for r in range(0, GR, RB)]

    def o_mm(g, last):
        return proj("p", g, "m", "o", last and g < NG - 1, o_rows(g, last))

    def o_rows(g, last):
        def step(r):
            x = st["res", g, r] + st["o", g, r]
            if last:
                for i in range(0, RB, G):
                    xio[g, (r + i) // G] = x[i:i + G].astype(BF16)
                if (r + RB) % HR == 0:
                    o_copy(g, r // HR).start()
            else:
                st["res", g, r] = x
                fwd_rows(g, r, x)
        return [partial(step, r) for r in range(0, GR, RB)]

    def fence():
        pl.semaphore_signal(bsem)
        pl.semaphore_wait(bsem)

    def at(f, g, *a):
        return f(g, *a) if 0 <= g < NG else []

    def rows(c):
        t = _r10_fwd(_tiles(load_x(c, 0, GR)), None, None, partial(_ln_r5, centred=True))
        for j in range(NT):
            ybuf[j] = t[j]

    def cols(c):
        for j in range(NT):
            st["y", NG, j] = d5(lambda i: ybuf[i], _F5, j)
        return s_fwd(NG, G * c)

    def filt(c):
        w_copy(0, c).wait()
        w_copy(1, c).wait()
        return sum([prep_filter(c, t) for t in range(WL // 128)], [])

    def w_start(c):
        w_copy(0, c).start()
        w_copy(1, c).start()

    def first(c, _):
        x_copy(c).wait()
        pl.when(c + AHEAD < NG)(lambda: x_copy(c + AHEAD).start())
        pl.when(c == NG - 2)(lambda: m_copy(1).start())
        for i in range(NW):
            pl.when(c == NG - NW + i)(partial(w_start, i))
        _run([partial(rows, c)], cols(c - 1))

    x_copy(0).start()
    m_copy(0).start()
    x_copy(1).start()
    x_copy(0).wait()
    for c in range(2, AHEAD + 1):
        x_copy(c).start()
    rows(0)
    m_copy(0).wait()
    lax.fori_loop(1, NG, first, None)

    order = list(range(1, 16)) + [0]
    for c in range(NW):
        if c == 1:
            m_copy(1).wait()
        pf = filt(c)
        if c == 0:
            m_copy(2).start()
        if c == NW - 1:
            m_copy(3).start()
            for j in range(NT):
                a_copy(1, j).start()
        _run(pf, [partial(mid_fwd, s) for s in order[6 * c - 6:6 * c]] if c else cols(NG - 1))
    m_copy(2).wait()

    nop = lambda: None
    for layer in range(2):
        for g in range(NG):
            st.pop(("xn", g), None)
            st.pop(("p", g), None)
        for i in range(16 + LAG):
            if layer == 0 and i == 2:
                prep_filter_end()
            if layer == 0 and i == 15 + LAG:
                m_copy(3).wait()
                for j in range(NT):
                    a_copy(1, j).wait()
                m_copy(4).start()
            if layer and i < 16:
                mid_fwd(order[i])
            if i >= LAG:
                mid_bwd(order[i - LAG])
            if i < 16:
                mid_filter(order[i])
        fence()
        for g in range(NG + 2):
            if layer == 0:
                if g == 0:
                    for j in range(NT):
                        prep_wk(j)
                if 1 <= g <= NT:
                    wqkv[0, 128 * g - 128:128 * g - 112, :128] = (
                        st["xn", g - 1, 0][:, :128].astype(BF16))
                    for k in (0, 2, 3):
                        a_copy(k, g - 1).start()
                if g == NG:
                    m_copy(4).wait()
                    for k in (0, 2, 3):
                        for j in range(NT):
                            a_copy(k, j).wait()
                    prep_wq(0)
                if g == NG + 1:
                    prep_wq(1)
                    prep_wq(2)
            _run(at(s_bwd, g))
            _run(at(d_bwd, g) + [nop] * 5, at(g_mm, g - 2), at(k_mm, g - 1))
        if layer:
            fence()
        mix_z()
        _run(q_mm(0))
        mix_kv()
        mix_m()
        _run(q_mm(1))
        for g in range(NG + 1):
            dm = [] if layer else _zip(at(d_fwd, g - 1), at(s_fwd, g - 1))
            _run((at(q_mm, g + 1) if g else []) + at(o_mm, g, layer == 1),
                 [nop] * 14 + dm)
    for c in range(NG):
        o_copy(c, 0).wait()
        o_copy(c, 1).wait()


@jax.jit
def pallas_interleave_layers__spectral_gfnet__linear_attn_block__prompt_kernel(
    A_x, A_w_r, A_w_i, B_x, B_wqkv, B_wo
):
    del B_x
    vm = pltpu.VMEM
    out = pl.pallas_call(
        _kernel,
        in_specs=[pl.BlockSpec(memory_space=pl.ANY)] * 6,
        out_specs=pl.BlockSpec(memory_space=pl.ANY),
        out_shape=jax.ShapeDtypeStruct((R1, R2, D), BF16),
        scratch_shapes=[
            vm((NG, R1, G, D), BF16),
            vm((NT, GR, 128), F32),
            vm((16, R2, D), I32),
            vm((2, S // WL, DF, WL), BF16),
            vm((NW, WL // 128, 2, D // 4 + 8, 128), I32),
            vm((3, R1 * PITCH + R2, 128), I32),
            vm((3, D, D), BF16),
            vm((D, D), BF16),
            vm((3, D + 24, 128), I32),
            vm((D + 24, 128), F32),
            vm((NT, D + 24, 128), F32),
            vm(_MATS.shape, I32),
            pltpu.SemaphoreType.DMA((10,)),
            pltpu.SemaphoreType.REGULAR,
        ],
        compiler_params=pltpu.CompilerParams(vmem_limit_bytes=100 * 1024 * 1024),
    )(A_x.reshape(R1, R2, D), A_w_r.T, A_w_i.T, B_wqkv, B_wo, _MATS)
    return out.reshape(1, S, D)
```

```python
from functools import partial

import numpy as np
import jax
import jax.numpy as jnp
from jax import lax
import jax.experimental.pallas as pl
import jax.experimental.pallas.tpu as pltpu

S, D, H, DH = 2048, 640, 32, 20
DF = D // 2 + 1
R1, R2 = 32, 64
G = 8
NG = R2 // G
GR = R1 * G
NT = D // 128

_C5 = float(np.sqrt(5.0) / 4.0)
_R5 = float(np.sin(4 * np.pi / 5) / np.sin(2 * np.pi / 5))
_PAIRS = ((0, 0), (1, 1), (2, 1), (1, 2), (2, 2), (3, 3), (4, 3), (3, 4), (4, 4))
_CLASSES = ((0, 5), (4, 6), (1, 9), (2, 8), (3, 7))


def _cmul(re, im, ang):
    c, s = float(np.cos(ang)), float(np.sin(ang))
    if abs(abs(c) - abs(s)) < 1e-12:
        if c * s > 0:
            return (re - im) * c, (re + im) * c
        return (re + im) * c, (im - re) * c
    return re * c - im * s, re * s + im * c


def _cadd(p, q):
    return p[0] + q[0], p[1] + q[1]


def _csub(p, q):
    return p[0] - q[0], p[1] - q[1]


def _cplx_fwd(u, th):
    n = len(u)
    if n == 1:
        return [(th, u[0])]
    if n == 4:
        v1, v2, v3 = (_cmul(*u[k], k * th / 4) for k in (1, 2, 3))
        a, b, c, d = _cadd(u[0], v2), _csub(u[0], v2), _cadd(v1, v3), _csub(v1, v3)
        out = _cadd(a, c), _csub(a, c), (b[0] - d[1], b[1] + d[0]), (b[0] + d[1], b[1] - d[0])
        return [(th / 4 + k * np.pi / 2, o) for k, o in zip((0, 2, 1, 3), out)]
    h = n // 2
    v = [_cmul(re, im, th / 2) for re, im in u[h:]]
    a = [_cadd(p, q) for p, q in zip(u[:h], v)]
    b = [_csub(p, q) for p, q in zip(u[:h], v)]
    return _cplx_fwd(a, th / 2) + _cplx_fwd(b, th / 2 + np.pi)


def _cplx_bwd(g, th):
    n = len(g)
    if n == 1:
        return list(g)
    if n == 4:
        a, c, b = _cadd(g[0], g[1]), _csub(g[0], g[1]), _cadd(g[2], g[3])
        d = (g[2][1] - g[3][1], g[3][0] - g[2][0])
        v = _cadd(c, d), _csub(a, b), _csub(c, d)
        return [_cadd(a, b)] + [_cmul(*v[k - 1], -k * th / 4) for k in (1, 2, 3)]
    h = n // 2
    a, b = _cplx_bwd(g[:h], th / 2), _cplx_bwd(g[h:], th / 2 + np.pi)
    return [_cadd(p, q) for p, q in zip(a, b)] + [
        _cmul(*_csub(p, q), -th / 2) for p, q in zip(a, b)]


def _real_fwd(x):
    n = len(x)
    if n == 2:
        return [(0.0, (x[0], x[1]))]
    h, q = n // 2, n // 4
    a = [x[j] + x[j + h] for j in range(h)]
    b = [x[j] - x[j + h] for j in range(h)]
    return _real_fwd(a) + _cplx_fwd([(b[j], b[j + q]) for j in range(q)], np.pi / 2)


def _real_bwd(g):
    if len(g) == 1:
        return list(g[0])
    h = len(g) // 2
    a = _real_bwd(g[:h])
    u = _cplx_bwd(g[h:], np.pi / 2)
    b = [p[0] for p in u] + [p[1] for p in u]
    return [p + q for p, q in zip(a, b)] + [p - q for p, q in zip(a, b)]


def _r10_fwd(x, sel, roll, norm=None):
    if sel is not None:
        x = [sel(x[j], x[(j + 2) % 5]) for j in range(5)]
    t1, t2, t3, t4 = x[1] + x[4], x[2] + x[3], x[1] - x[4], x[2] - x[3]
    t5 = t1 + t2
    y0, m1, m2 = x[0] + t5, x[0] - t5 * 0.25, (t1 - t2) * _C5
    out = []
    for re, im in ((m1 + m2, t3 + t4 * _R5), (m1 - m2, t3 * _R5 - t4)):
        if sel is None:
            out += [re, im]
        else:
            a, b = sel(re, im), roll(sel(im, re))
            out += [a + b, a - b]
    if norm is None:
        return [y0] + out
    y0, scale = norm(y0, m1, m2, t3, t4)
    return [a * scale for a in [y0] + out]


def _r10_bwd(g, sel, roll):
    re, im = [], []
    for u, v in ((g[1], g[2]), (g[3], g[4])):
        a, b = u + v, roll(u - v)
        re.append(sel(a, b))
        im.append(sel(b, a))
    m1, e = re[0] + re[1], (re[0] - re[1]) * _C5
    t5 = g[0] - m1 * 0.25
    t1, t2 = t5 + e, t5 - e
    t3, t4 = im[0] + im[1] * _R5, im[0] * _R5 - im[1]
    x = [g[0] + m1, t1 + t3, t2 + t4, t2 - t4, t1 - t3]
    return [sel(x[j], x[(j + 3) % 5]) for j in range(5)]


def _build_constants():
    lane = np.arange(128)
    grp = [np.concatenate([c + 10 * np.arange(32) for c in cls]) for cls in _CLASSES]
    d = np.arange(D)[:, None]
    cols = []
    for g, kd in enumerate(grp):
        c, s = np.cos(2 * np.pi * d * kd / D), np.sin(2 * np.pi * d * kd / D)
        if g == 0:
            s[:, 0] = np.cos(np.pi * d[:, 0])
        cols.append(np.concatenate([s, c] if g in (2, 4) else [c, s], axis=1))
    eye = np.eye(D)
    net = np.concatenate(_r10_fwd(
        [eye[:, 128 * j:128 * j + 128] for j in range(NT)],
        lambda a, b: np.where(lane < 64, a, b), lambda a: np.roll(a, 64, axis=1)), axis=1)
    bd = np.linalg.solve(net, np.concatenate(cols, axis=1))
    fd = np.stack([bd[128 * j:128 * j + 128, 128 * j:128 * j + 128] for j in range(NT)])
    assert abs(np.abs(bd).sum() - np.abs(fd).sum()) < 1e-6
    dmat = np.concatenate([fd, fd.transpose(0, 2, 1) / D])
    dmat[NT, ::64] *= 0.5

    cs = [cols[0]] + [np.concatenate(p, axis=1) for j in (1, 3) for p in (
        (cols[j][:, :64], cols[j + 1][:, 64:]), (cols[j][:, 64:], cols[j + 1][:, :64]))]
    net = np.concatenate(_r10_fwd(
        [eye[:, 128 * j:128 * j + 128] for j in range(NT)], None, None), axis=1)
    bd = np.linalg.solve(net, np.concatenate(cs, axis=1))
    f5 = np.stack([bd[128 * i:128 * i + 128, 128 * j:128 * j + 128] for i, j in _PAIRS])
    assert abs(np.abs(bd).sum() - np.abs(f5).sum()) < 1e-6

    leaves = [int(round(th * R1 / (2 * np.pi))) for th, _ in _real_fwd(list(np.eye(R1)))]
    k1 = [min(m, R1 - m) for m in leaves]
    pos = np.arange(128)
    part, n2 = (pos // G) % 2, (pos // (2 * G)) * G + pos % G
    fs = []
    for m, kk in zip(leaves, k1):
        ks = (16 * np.arange(R2) if m == 0 else kk + R1 * np.arange(R2))[:, None]
        if m == 0:
            ph = 2 * np.pi * ks * (n2 + R2 * part) / S
            c, s = np.cos(ph), np.sin(ph)
            s[0] = np.cos(np.pi * n2)
        else:
            sg = 1.0 if m == kk else -1.0
            ph = 2 * np.pi * ks * n2 / S
            c = np.where(part == 0, np.cos(ph), -sg * np.sin(ph))
            s = np.where(part == 0, np.sin(ph), sg * np.cos(ph))
        fs.append(np.concatenate([c, s]))
    fs = np.stack(fs)[:, part * R2 + n2]
    smat = np.concatenate([fs, fs.transpose(0, 2, 1) * (2.0 / S)])

    have = np.concatenate([R1 * np.arange(R2), 16 + R1 * (R2 - 1 - np.arange(R2))])
    want = np.concatenate([16 * np.arange(R2), S // 2 + 16 * ((R2 - np.arange(R2)) % R2)])
    p0 = (want[:, None] == have[None, :]).astype(np.float64)

    mats = np.concatenate([f5, smat, p0[None], dmat[NT:], dmat[:NT]]).astype(jnp.bfloat16)
    mats = mats.view(np.uint16).astype(np.uint32)
    return (mats[:, 0::2] | (mats[:, 1::2] << 16)).view(np.int32), k1


_MATS, _K1 = _build_constants()
_F5, _SF, _SI, _P0, _DI, _DF, _NM = 0, 9, 25, 41, 42, 47, 52

F32, BF16, I32 = jnp.float32, jnp.bfloat16, jnp.int32
PITCH = 68
RB = 16
HR = GR // 2
KB = 160
NW = 4
WL = S // NW
LAG = 2
AHEAD = 3
F5 = 7
_MCUT = (0, _SF, _SI, _DI, _DF, _NM)
_HI = np.int32(-65536)
_WIN = ((0, 144), (112, 272), (240, 400), (368, 528), (496, 640))


def _dot(a, b):
    return jnp.dot(a.astype(BF16), b.astype(BF16), preferred_element_type=F32)


def _dot_nt(a, b):
    return lax.dot_general(a.astype(BF16), b.astype(BF16), (((1,), (1,)), ((), ())), preferred_element_type=F32)


def _sel(a, b):
    return jnp.where(lax.broadcasted_iota(I32, a.shape, 1) < 64, a, b)


def _roll(a):
    return pltpu.roll(a, 64, 1)


def _tiles(a):
    return [a[:, 128 * j:128 * j + 128] for j in range(a.shape[1] // 128)]


def _cat(a, axis=0):
    return a[0] if len(a) == 1 else jnp.concatenate(a, axis=axis)


def _split(a):
    return [_cat([a[r:r + G] for r in range(o, a.shape[0], 2 * G)]) for o in (0, G)]


def _merge(a, b):
    return _cat([x[r:r + G] for r in range(0, a.shape[0], G) for x in (a, b)])


def _quads(a, h, w):
    return a[:h, :w], a[:h, w:2 * w], a[h:2 * h, :w], a[h:2 * h, w:2 * w]


def _terms_a(a11, a12, a21, a22):
    return a11 + a22, a22 - a21, a11, a22, a11 - a12, a21 + a11, a12 + a22


def _terms_w(w11, w12, w21, w22):
    return w11 + w22, w11, w12 + w22, w21 + w11, w22, w12 - w11, w21 - w22


_USE = (((0, 1), (3, 1)), ((2, -1), (3, -1)), ((1, 1), (3, -1)), ((0, -1), (2, 1)),
        ((0, -1), (1, -1)), ((3, 1),), ((0, 1),))
_ORD = (6, 4, 0, 3, 1, 2, 5)
_GORD = (0, 1, 6, 2, 3, 4, 5, 7, 8)


def _combine(c, p):
    c = list(c)
    for i in reversed(_ORD):
        for k, sg in _USE[i]:
            c[k] = c[k] + p[i] if sg > 0 else c[k] - p[i]
    return c


def _unpack(w):
    return pltpu.bitcast(w & _HI, F32), pltpu.bitcast(w << 16, F32)


def _words(a):
    return pltpu.bitcast(a, I32)


def _phi(t):
    return jnp.where(t > 0, t + 1.0, jnp.exp(t)) + 1e-6


def _ln(x):
    mean = _lane_sum(x[0] + x[1] + x[2] + x[3] + x[4]) * (1.0 / D)
    sq = _lane_sum(x[0] * x[0] + x[1] * x[1] + x[2] * x[2] + x[3] * x[3] + x[4] * x[4])
    r = lax.rsqrt(jnp.maximum(sq * (1.0 / D) - mean * mean, 0.0) + 1e-5)
    return [(a - mean) * r for a in x]


def _lane_sum(a):
    return jnp.sum(a, axis=1, keepdims=True)


def _ln_r5(y0, m1, m2, t3, t4, centred=False):
    mean = _lane_sum(y0) * (1.0 / 128)
    yc = y0 - mean
    sq = (m1 * m1 + m2 * m2) * 4.0 + (t3 * t3 + t4 * t4) * 2.5
    if centred:
        var = _lane_sum(sq + yc * yc) * (0.2 / D)
    else:
        var = jnp.maximum(_lane_sum(sq + y0 * y0) * (0.2 / D) - mean * mean * 0.04, 0.0)
    return yc, lax.rsqrt(var + 1e-5)


def _bf(a):
    return pltpu.bitcast(a, BF16)


def _run(*gens):
    gens = [list(g) for g in gens]
    order = sorted(((i + 0.5) / len(g), k, i) for k, g in enumerate(gens) for i in range(len(g)))
    for _, k, i in order:
        gens[k][i]()


def _zip(a, b):
    n = len(b) // max(len(a), 1)
    return [f for i, p in enumerate(a) for f in [p] + b[i * n:i * n + n]]


def _ds(start, size, align=None):
    if isinstance(start, int):
        return pl.ds(start, size)
    return pl.ds(pl.multiple_of(start, align or size), size)


def _kernel(x_hbm, wr_hbm, wi_hbm, wqkv_hbm, wo_hbm, mats_hbm, o_hbm,
            xio, ybuf, z0, wraw, wtmp, wbuf, wqkv, wo, wqt, zacc, macc, mats, sems, bsem):

    def x_copy(c):
        return pltpu.make_async_copy(x_hbm.at[:, _ds(G * c, G), :], xio.at[c], sems.at[c & 3])

    def o_copy(c, h):
        n1 = pl.ds(h * (R1 // 2), R1 // 2)
        return pltpu.make_async_copy(xio.at[c, n1], o_hbm.at[n1, _ds(G * c, G), :], sems.at[0])

    def w_copy(i, c):
        return pltpu.make_async_copy(
            (wr_hbm, wi_hbm)[i].at[:, _ds(WL * c, WL)], wraw.at[i, c], sems.at[6 + c % 4])

    def m_copy(i):
        lo, hi = _MCUT[i], _MCUT[i + 1]
        return pltpu.make_async_copy(mats_hbm.at[lo:hi], mats.at[lo:hi], sems.at[4 + i % 2])

    def a_copy(k, i):
        rs = pl.ds(128 * i, 128)
        if k == 3:
            return pltpu.make_async_copy(wo_hbm.at[rs], wo.at[rs], sems.at[2])
        return pltpu.make_async_copy(
            wqkv_hbm.at[rs, pl.ds(D * k, D)], wqkv.at[k, rs], sems.at[1 if k == 1 else 2])

    mat = lambda i: _bf(mats[i])
    st = {}

    def fwd_rows(g, r, x):
        st["t", g, r] = _r10_fwd(_tiles(x), _sel if g < F5 else None, _roll, _ln_r5)

    def d5(t, base, j):
        ks = [k for k, p in enumerate(_PAIRS) if p[1] == j]
        return _dot(_cat([t(_PAIRS[k][0]) for k in ks], 1),
                    _cat([mat(base + k) for k in ks]))

    def load_x(g, r, n):
        return _cat([xio[g, i].astype(F32) for i in range(r // G, (r + n) // G)])

    def d_fwd(g):
        def step(j):
            t = lambda i: _cat([st["t", g, r][i] for r in range(0, GR, RB)])
            st["y", g, j] = _dot(t(j).astype(BF16), mat(_DF + j)) if g < F5 else d5(t, _F5, j)
        return [partial(step, j) for j in range(NT)]

    def s_fwd(g, row=None):
        def put(s, j, w):
            if row is None:
                st["z", s, g, j] = w
            else:
                z0[s, _ds(row, G), 128 * j:128 * j + 128] = w

        def step(j):
            y = st["y", g, j]
            v = _real_fwd([y[n * G:n * G + G, :] for n in range(R1)])
            w = [_words(_merge(*p).astype(BF16)) for _, p in v]
            st["w", g, j] = w
            for s in range(16):
                if j == 0 or g >= F5:
                    put(s, j, w[s])
                elif j % 2 == 0:
                    a, b = st["w", g, j - 1][s], w[s]
                    put(s, j - 1, _sel(a, b))
                    put(s, j, _roll(_sel(b, a)))
        return [partial(step, j) for j in range(NT)]

    def s_bwd(g):
        def step(j):
            r0 = 2 * G * g
            w = _cat(_real_bwd([(st["zi", s, j][r0:r0 + G], st["zi", s, j][r0 + G:r0 + 2 * G])
                                for s in range(16)]))
            st["u", g, j] = w
        return [partial(step, j) for j in range(NT)]

    def d_bwd(g):
        def step(r, j):
            st["v", g, j] = _dot(st["u", g, j][r:r + HR], mat(_DI + j))
            if j == NT - 1:
                _run(bwd_rows(g)[r // RB:(r + HR) // RB])
        return [partial(step, r, j) for r in (0, HR) for j in range(NT)]

    def bwd_rows(g):
        def step(r):
            d = _r10_bwd([st["v", g, j][r % HR:r % HR + RB] for j in range(NT)],
                         _sel, _roll)
            x = st["res", g, r] if ("res", g, r) in st else load_x(g, r, RB)
            x = [a + b for a, b in zip(_tiles(x), d)]
            st["res", g, r] = _cat(x, 1)
            st["xn", g, r] = _cat(_ln(x), 1)
        return [partial(step, r) for r in range(0, GR, RB)]

    def prep_filter(c, t):
        ls = slice(128 * t, 128 * t + 128)

        def merge():
            a, b = _words(wraw[0, c, 0:D // 2, ls]), _words(wraw[1, c, 0:D // 2, ls])
            wtmp[c, t, 0, :D // 4] = (a << 16) | (b & 0xFFFF)
            wtmp[c, t, 1, :D // 4] = (a & _HI) | lax.shift_right_logical(b, 16)

        def step(j):
            cls = lambda k: wtmp[c, t, k % 2, pl.ds(k // 2, 32, stride=5), :]
            if j == 0:
                last = _words(wraw[0, c, D // 2:DF, ls].astype(F32)) | lax.shift_right_logical(
                    _words(wraw[1, c, D // 2:DF, ls].astype(F32)), 16)
                c0, c5 = cls(0), cls(5)
                src = [c0, c5, jnp.where(lax.broadcasted_iota(I32, c0.shape, 0) == 0, last, c0), c5]
            else:
                src = [cls(k) for k in _CLASSES[2 * j - 1] + _CLASSES[2 * j]]
            w = _cat(src).T
            for i in range(16):
                k2, k1 = (WL // R1) * c + 4 * t + i // 4, 8 * (i % 4)
                pos = k2 if k1 < 16 else R2 - 1 - k2
                wbuf[j, pl.ds(k1 * PITCH + pos, 8, stride=PITCH), :] = w[8 * i:8 * i + 8]
        return [merge] + [partial(step, j) for j in range(3)]

    def prep_filter_end():
        for j in range(3):
            w = _cat([wbuf[j, 0:R2, :], wbuf[j, 16 * PITCH:16 * PITCH + R2, :]])
            re = _dot(mat(_P0), pltpu.bitcast(w & _HI, F32).astype(BF16))
            im = _dot(mat(_P0), pltpu.bitcast(w << 16, F32).astype(BF16))
            w = _words(re) | lax.shift_right_logical(_words(im), 16)
            wbuf[j, 0:R2, :] = w[:R2]
            wbuf[j, 16 * PITCH:16 * PITCH + R2, :] = w[R2:]

    def prep_wq(i):
        r0 = (0, 256, 384)[i]
        wqt[i, :D] = _words(wqkv[0, r0:r0 + 256, :]).T
        w = _cat([wqt[i, pl.ds(d, H, stride=DH), :] for d in range(DH)]).T
        st["wq", i] = _bf(w[64:] if i == 2 else w)
        if i == 2:
            w = _cat([st["wq", k] for k in range(3)])
            st["wqs"] = w, _terms_w(*_quads(w.astype(F32), 256, 256))

    def prep_wk(j):
        for k in (0, 2, 1, 3, 4):
            w = wqkv[1, 128 * k:128 * k + 128, 128 * j:128 * j + 128]
            st["wk", j, k] = w.astype(F32).T
        if j == NT - 1:
            w = _cat([_cat([st["wk", i, k][o:o + 64] for k in range(NT)], 1)
                      for o in (0, 64) for i in range(NT)])
            w11, w21, w12, w22 = _quads(w, D // 2, 256)
            st["wkt"], st["wks"] = w, _terms_w(w11, w12, w21, w22)

    def natural(a):
        return _cat([a[o + 64 * i:o + 64 * i + 64] for i in range(NT) for o in (0, D // 2)])

    def masks(s):
        lane = lax.broadcasted_iota(I32, (R2, 128), 1)
        sign = jnp.where((lane & 63) == 0, 0.0, jnp.where(lane < 64, -1.0, 1.0))
        if s:
            return lane, sign, lambda a: a
        row = lax.broadcasted_iota(I32, (R2, 128), 0)
        return lane, sign, lambda a: jnp.where(row == 0, 0.0, a)

    def mid_fwd(s):
        x = []
        for j in range(NT):
            if ("z", s, 0, j) in st:
                a = _cat([st["z", s, g, j] for g in range(NG)])
            else:
                a = z0[s, :, 128 * j:128 * j + 128]
            x.append(_split(_dot(mat(_SF + s), _bf(a))))
        _, sign, m = masks(s)
        st["x", s, 0] = _sel(*x[0]), _sel(*x[0][::-1])
        for j in (1, 3):
            (cc, sc), (cs, ss) = x[j], x[j + 1]
            st["x", s, j] = cc - m(ss), cs + m(sc), m(cc) + ss, m(cs) - sc

    def mid_filter(s):
        k1 = _K1[s]
        p1, p2 = k1 * PITCH, (R1 - k1 if k1 else 16) * PITCH
        lane, sign, m = masks(s)
        a, b = st["x", s, 0]
        re, im = a + m(_roll(a) * sign), m(b) - _roll(b) * sign
        w1, w2 = wbuf[0, p1:p1 + R2, :], wbuf[0, p2:p2 + R2, :]
        (a1, b1), (a2, b2) = _unpack(_sel(w1, w2)), _unpack(
            jnp.where(lane == 0, w2, jnp.where(lane == 64, w1, 0)))
        cr, ci = a1 + a2, b1 - b2
        re, im = cr * re + ci * im, cr * im - ci * re
        an, bn = re - m(_roll(re) * sign), m(im) + _roll(im) * sign
        if not k1:
            corner = (lax.broadcasted_iota(I32, a.shape, 0) + (lane & 63)) == 0
            an, bn = jnp.where(corner, a * a1, an), jnp.where(corner, b * a2, bn)
        out = [_merge(_sel(an, bn), _sel(bn, an))]
        for j in (1, 3):
            r1, n1, r2, n2 = st["x", s, j]
            (a1, b1), (a2, b2) = (_unpack(wbuf[(j + 1) // 2, p:p + R2, :]) for p in (p1, p2))
            r1, n1 = a1 * r1 + b1 * n1, a1 * n1 - b1 * r1
            r2, n2 = a2 * r2 + b2 * n2, a2 * n2 - b2 * r2
            a, b = _merge(r1 + m(r2), m(n1) - n2), _roll(_merge(n1 + m(n2), r2 - m(r1)))
            out += [_sel(a, b), _sel(b, a)]
        st["f", s] = out

    def mid_bwd(s):
        for j in range(NT):
            st["zi", s, j] = _dot(mat(_SI + s), st["f", s][j])

    def half(name, h):
        if name != "xn":
            return range(h * HR, h * HR + HR, RB)
        return range(h * RB, GR, 2 * RB)

    def terms(name, g):
        if (name, g) not in st:
            a = _cat([st[name, g, r] for h in (0, 1) for r in half(name, h)])
            st[name, g] = a, _terms_a(*_quads(a, HR, 256))
        return st[name, g]

    def proj(name, g, w, out, fast, then):
        def put(o, y):
            for i, r in enumerate(half(name, o)):
                st[out, g, r] = y[i * RB:i * RB + RB]

        def plain(h):
            put(h, _dot(terms(name, g)[0][h * HR:h * HR + HR], st[w][0]))
            _run([then[r // RB] for r in half(name, h)])

        def side():
            st["e", out] = _dot(terms(name, g)[0], st[w][0][:, 512:])

        def edge():
            c = _dot(terms(name, g)[0][:, 512:], st[w][0][512:, :512])
            c = _combine(_quads(c, HR, 256), [st["c", out, i] for i in range(7)])
            put(0, _cat([c[0], c[1], st["e", out][:HR]], 1))
            put(1, _cat([c[2], c[3], st["e", out][HR:]], 1))
            _run(then)

        def step(i):
            st["c", out, i] = _dot(terms(name, g)[1][i], st[w][1][i])
        if not fast:
            return [partial(plain, h) for h in (0, 1)]
        return [side] + [partial(step, i) for i in _ORD] + [edge]

    def k_mm(g):
        def edge(r):
            e = [_dot_nt(st["wkt"][o:o + KB, 512:], terms("xn", g)[0][:, 512:])
                 for o in (r, D // 2 + r)]
            c = _combine([e[0][:, :HR], e[1][:, :HR], e[0][:, HR:], e[1][:, HR:]],
                         [st["ck", i] for i in range(7)])
            c = [_phi(a) for a in c]
            for o, zs in ((r, c[0] + c[2]), (D // 2 + r, c[1] + c[3])):
                st["zs", o] = st["zs", o] + zs if g else zs
            st["pk", g, r] = ([_cat(c[i::2], 1) for i in (0, 1)],
                              _terms_a(c[0], c[2], c[1], c[3]))

        def step(r, i):
            st["ck", i] = _dot_nt(st["wks"][i][r:r + KB], terms("xn", g)[1][i])
        return [f for r in range(0, D // 2, KB)
                for f in [partial(step, r, i) for i in _ORD] + [partial(edge, r)]]

    def g_mm(g):
        def step(r, i):
            if i < 7:
                a = _dot(st["pk", g, r][1][i], terms("xn", g)[1][(0, 2, 6, 5, 3, 4, 1)[i]])
            else:
                a = _dot(st["pk", g, r][0][i - 7], terms("xn", g)[0][:, 512:])
            st["g", r, i] = st["g", r, i] + a if g else a
        return [partial(step, r, i) for r in range(0, D // 2, KB) for i in _GORD]

    def mix_z():
        zacc[:D] = natural(_cat([st["zs", r] for r in range(0, D, KB)]))
        zp = _cat([zacc[pl.ds(d, H, stride=DH), :] for d in range(DH)])
        st["zrow"] = jnp.broadcast_to(jnp.sum(zp.T, axis=0, keepdims=True), (RB, D))

    def mix_kv():
        m1, m2, n3, n4, m5, n6, n7, e0, e1 = (
            _cat([st["g", r, i] for r in range(0, D // 2, KB)]) for i in range(9))
        gm = natural(_cat([_cat([m1 - n4 - m5 - n7, n3 - m5, e0], 1),
                           _cat([n4 - m2, m1 - m2 - n3 - n6, e1], 1)]))
        for j, (r0, r1) in enumerate(_WIN):
            kv = _dot(gm[r0:r1], wqkv[2, :, 128 * j:128 * j + 128])
            hr = ((lax.broadcasted_iota(I32, kv.shape, 0) + r0) * 3277) >> 16
            hc = ((lax.broadcasted_iota(I32, kv.shape, 1) + 128 * j) * 3277) >> 16
            st["kv", j] = jnp.where(hr == hc, kv, 0.0).astype(BF16)

    def mix_m():
        done = 0
        for j, (r0, r1) in enumerate(_WIN):
            m = _dot(st["kv", j], wo[128 * j:128 * j + 128, :])
            for t, a in enumerate(_tiles(m)):
                if done > r0:
                    macc[t, r0:done, :] += a[:done - r0]
                macc[t, done:r1, :] = a[done - r0:]
            done = r1
        w = _cat([_cat([macc[t, pl.ds(d, H, stride=DH), :] for d in range(DH)])
                  for t in range(NT)], 1)
        st["m"] = w, _terms_w(*_quads(w, 256, 256))

    def q_mm(g):
        return proj("xn", g, "wqs", "q", True, q_act(g))

    def q_act(g):
        def step(r):
            zt = _tiles(st["zrow"])
            p = _tiles(_phi(st["q", g, r]))
            den = p[0] * zt[0] + p[1] * zt[1] + p[2] * zt[2] + p[3] * zt[3] + p[4] * zt[4]
            den = den + _roll(den)
            den = den + pltpu.roll(den, 32, 1)
            den = den + 1e-6
            inv = pl.reciprocal(den, approx=True)
            inv = inv * (2.0 - den * inv)
            st["p", g, r] = _cat([a * inv for a in p], 1)
        return [partial(step, r) for r in range(0, GR, RB)]

    def o_mm(g, last):
        return proj("p", g, "m", "o", last and g < NG - 1, o_rows(g, last))

    def o_rows(g, last):
        def step(r):
            x = st["res", g, r] + st["o", g, r]
            if last:
                for i in range(0, RB, G):
                    xio[g, (r + i) // G] = x[i:i + G].astype(BF16)
                if (r + RB) % HR == 0:
                    o_copy(g, r // HR).start()
            else:
                st["res", g, r] = x
                fwd_rows(g, r, x)
        return [partial(step, r) for r in range(0, GR, RB)]

    def fence():
        pl.semaphore_signal(bsem)
        pl.semaphore_wait(bsem)

    def at(f, g, *a):
        return f(g, *a) if 0 <= g < NG else []

    def rows(c):
        t = _r10_fwd(_tiles(load_x(c, 0, GR)), None, None, partial(_ln_r5, centred=True))
        for j in range(NT):
            ybuf[j] = t[j]

    def cols(c):
        for j in range(NT):
            st["y", NG, j] = d5(lambda i: ybuf[i], _F5, j)
        return s_fwd(NG, G * c)

    def filt(c):
        w_copy(0, c).wait()
        w_copy(1, c).wait()
        return sum([prep_filter(c, t) for t in range(WL // 128)], [])

    def w_start(c):
        w_copy(0, c).start()
        w_copy(1, c).start()

    def first(c, _):
        x_copy(c).wait()
        pl.when(c + AHEAD < NG)(lambda: x_copy(c + AHEAD).start())
        pl.when(c == NG - 2)(lambda: m_copy(1).start())
        for i in range(NW):
            pl.when(c == NG - NW + i)(partial(w_start, i))
        _run([partial(rows, c)], cols(c - 1))

    x_copy(0).start()
    m_copy(0).start()
    x_copy(1).start()
    x_copy(0).wait()
    for c in range(2, AHEAD + 1):
        x_copy(c).start()
    rows(0)
    m_copy(0).wait()
    lax.fori_loop(1, NG, first, None)

    order = list(range(1, 16)) + [0]
    for c in range(NW):
        if c == 1:
            m_copy(1).wait()
        pf = filt(c)
        if c == 0:
            m_copy(2).start()
        if c == NW - 1:
            m_copy(3).start()
            for j in range(NT):
                a_copy(1, j).start()
        _run(pf, [partial(mid_fwd, s) for s in order[6 * c - 6:6 * c]] if c else cols(NG - 1))
    m_copy(2).wait()

    nop = lambda: None
    for layer in range(2):
        for g in range(NG):
            st.pop(("xn", g), None)
            st.pop(("p", g), None)
        for i in range(16 + LAG):
            if layer == 0 and i == 2:
                prep_filter_end()
            if layer == 0 and i == 15 + LAG:
                m_copy(3).wait()
                for j in range(NT):
                    a_copy(1, j).wait()
                m_copy(4).start()
            if layer and i < 16:
                mid_fwd(order[i])
            if i >= LAG:
                mid_bwd(order[i - LAG])
            if i < 16:
                mid_filter(order[i])
        fence()
        for g in range(NG + 2):
            if layer == 0:
                if g == 0:
                    for j in range(NT):
                        prep_wk(j)
                if 1 <= g <= NT:
                    wqkv[0, 128 * g - 128:128 * g - 112, :128] = (
                        st["xn", g - 1, 0][:, :128].astype(BF16))
                    for k in (0, 2, 3):
                        a_copy(k, g - 1).start()
                if g == NG:
                    m_copy(4).wait()
                    for k in (0, 2, 3):
                        for j in range(NT):
                            a_copy(k, j).wait()
                    prep_wq(0)
                if g == NG + 1:
                    prep_wq(1)
                    prep_wq(2)
            _run(at(s_bwd, g))
            _run(at(d_bwd, g) + [nop] * 5, at(g_mm, g - 2), at(k_mm, g - 1))
        if layer:
            fence()
        mix_z()
        _run(q_mm(0))
        mix_kv()
        mix_m()
        _run(q_mm(1))
        for g in range(NG + 1):
            dm = [] if layer else _zip(at(d_fwd, g - 1), at(s_fwd, g - 1))
            _run((at(q_mm, g + 1) if g else []) + at(o_mm, g, layer == 1),
                 [nop] * 14 + dm)
    for c in range(NG):
        o_copy(c, 0).wait()
        o_copy(c, 1).wait()


@jax.jit
def pallas_interleave_layers__spectral_gfnet__linear_attn_block__prompt_kernel(
    A_x, A_w_r, A_w_i, B_x, B_wqkv, B_wo
):
    del B_x
    vm = pltpu.VMEM
    out = pl.pallas_call(
        _kernel,
        in_specs=[pl.BlockSpec(memory_space=pl.ANY)] * 6,
        out_specs=pl.BlockSpec(memory_space=pl.ANY),
        out_shape=jax.ShapeDtypeStruct((R1, R2, D), BF16),
        scratch_shapes=[
            vm((NG, R1, G, D), BF16),
            vm((NT, GR, 128), F32),
            vm((16, R2, D), I32),
            vm((2, S // WL, DF, WL), BF16),
            vm((NW, WL // 128, 2, D // 4 + 8, 128), I32),
            vm((3, R1 * PITCH + R2, 128), I32),
            vm((3, D, D), BF16),
            vm((D, D), BF16),
            vm((3, D + 24, 128), I32),
            vm((D + 24, 128), F32),
            vm((NT, D + 24, 128), F32),
            vm(_MATS.shape, I32),
            pltpu.SemaphoreType.DMA((10,)),
            pltpu.SemaphoreType.REGULAR,
        ],
        compiler_params=pltpu.CompilerParams(vmem_limit_bytes=100 * 1024 * 1024),
    )(A_x.reshape(R1, R2, D), A_w_r.T, A_w_i.T, B_wqkv, B_wo, _MATS)
    return out.reshape(1, S, D)
```
